```python
import jax
import jax.numpy as jnp

def _softmax(x, axis=-1):
    return jax.nn.softmax(x, axis=axis)

def _gelu(x):
    return jax.nn.gelu(x, approximate=True)

def _silu(x):
    return jax.nn.silu(x)

def _sigmoid(x):
    return jax.nn.sigmoid(x)

def _layernorm(x, axis=-1, eps=1e-05):
    m = jnp.mean(x, axis=axis, keepdims=True)
    v = jnp.var(x, axis=axis, keepdims=True)
    return (x - m) / jnp.sqrt(v + eps)

def _scatter_add(tgt, idx, src, axis=0):
    return tgt.at[idx].add(src)

def _segment_sum(src, seg, n):
    return jax.ops.segment_sum(src, seg, n)

class _Rng:

    def __init__(self, key):
        self._k = key

    def _next(self):
        self._k, sub = jax.random.split(self._k)
        return sub

    def normal(self, shape):
        return jax.random.normal(self._next(), shape, dtype=jnp.bfloat16)

    def randint(self, lo, hi, shape):
        return jax.random.randint(self._next(), shape, lo, hi, dtype=jnp.int32)

    def uniform(self, shape, lo=0.0, hi=1.0):
        return jax.random.uniform(self._next(), shape, jnp.bfloat16, lo, hi)

    def permutation(self, n):
        return jax.random.permutation(self._next(), n)
kernel_name = 'concat_heads__memory_aug_recurrent_mem_tr__sliding_local_dilated__prompt'

def setup_inputs():
    _rng = _Rng(jax.random.key(int.from_bytes(__import__("os").urandom(4), "little")))
    _w = lambda a: (lambda t: t.astype(jnp.bfloat16) if jnp.issubdtype(t.dtype, jnp.floating) else t)(jnp.asarray(a))

    def _A_setup():
        B, S, Dm = (1, 2048, 1024)
        H, Dh = (32, 128)
        M, seg = (8, 32)
        seg = min(seg, S)
        S = S // seg * seg
        return {'x': _w((lambda *s: _rng.normal(s) * 0.05)(B, S, Dm)), 'mem0': _w((lambda *s: _rng.normal(s) * 0.05)(B, M, Dm)), 'Wq': _w((lambda *s: _rng.normal(s) * 0.05)(Dm, H, Dh) * Dm ** (-0.5)), 'Wk': _w((lambda *s: _rng.normal(s) * 0.05)(Dm, H, Dh) * Dm ** (-0.5)), 'Wv': _w((lambda *s: _rng.normal(s) * 0.05)(Dm, H, Dh) * Dm ** (-0.5)), 'Wo': _w((lambda *s: _rng.normal(s) * 0.05)(H, Dh, Dm) * (H * Dh) ** (-0.5)), 'seg_len': seg}
    _A_in = _A_setup()

    def _B_setup():
        B, S, D = (1, 2048, 1024)
        return {'x': _w((lambda *s: _rng.normal(s) * 0.05)(B, S, D)), 'wqkv': _w((lambda *s: _rng.normal(s) * 0.05)(D, 3 * D)), 'wo': _w((lambda *s: _rng.normal(s) * 0.05)(D, D))}
    _B_in = _B_setup()
    return {'A_x': _A_in['x'], 'A_mem0': _A_in['mem0'], 'A_Wq': _A_in['Wq'], 'A_Wk': _A_in['Wk'], 'A_Wv': _A_in['Wv'], 'A_Wo': _A_in['Wo'], 'A_seg_len': _A_in['seg_len'], 'B_x': _B_in['x'], 'B_wqkv': _B_in['wqkv'], 'B_wo': _B_in['wo']}

def reference(A_x, A_mem0, A_Wq, A_Wk, A_Wv, A_Wo, A_seg_len, B_x, B_wqkv, B_wo):

    def _A_ref(x, mem0, Wq, Wk, Wv, Wo, seg_len):
        B, S, Dm = x.shape
        H, Dh = (Wq.shape[1], Wq.shape[2])
        M = mem0.shape[1]
        scale = Dh ** (-0.5)
        n_seg = S // seg_len
        L = M + seg_len
        idx = jnp.arange(L)
        mask = (idx[:, None] < M) | (idx[:, None] >= idx[None, :])
        mem = mem0
        outs = []
        for s in range(n_seg):
            xs = x[:, s * seg_len:(s + 1) * seg_len, :].copy()
            h = jnp.concatenate([mem, xs], axis=1)
            q = jnp.einsum('btd,dhe->bhte', h, Wq)
            k = jnp.einsum('btd,dhe->bhte', h, Wk)
            v = jnp.einsum('btd,dhe->bhte', h, Wv)
            scores = jnp.einsum('bhqe,bhke->bhqk', q, k) * scale
            scores = jnp.where(mask[None, None], scores, -1000000000.0)
            p = _softmax(scores, axis=-1)
            o = jnp.einsum('bhqk,bhke->bhqe', p, v)
            o = jnp.einsum('bhte,hed->btd', o, Wo)
            mem = o[:, :M, :].copy()
            outs.append(o[:, M:, :])
        return jnp.concatenate(outs, axis=1)

    def _B_ref(x, wqkv, wo):
        B, S, D = x.shape
        H = 32
        Dh = D // H
        W, dil = (8, 2)
        qkv = (lambda x, *d: x.transpose(*d))((x @ wqkv).reshape(B, S, 3, H, Dh), 2, 0, 3, 1, 4)
        q, k, v = (qkv[0], qkv[1], qkv[2])
        scale = Dh ** (-0.5)
        pos = jnp.arange(S)
        off = jnp.arange(W) * dil
        idx = pos[:, None] - off[None, :]
        mask = idx >= 0
        idx_c = jnp.where(mask, idx, 0).reshape(-1)
        kg = k[:, :, idx_c, :].reshape(B, H, S, W, Dh)
        vg = v[:, :, idx_c, :].reshape(B, H, S, W, Dh)
        logits = jnp.einsum('bhsd,bhswd->bhsw', q, kg) * scale
        logits = jnp.where(mask[None, None, :, :], logits, -1000000000.0)
        attn = _softmax(logits, axis=-1)
        o = jnp.einsum('bhsw,bhswd->bhsd', attn, vg)
        return (lambda x, *d: x.transpose(*d))(o, 0, 2, 1, 3).reshape(B, S, D) @ wo
    a = _A_ref(A_x, A_mem0, A_Wq, A_Wk, A_Wv, A_Wo, A_seg_len)
    b = _B_ref(B_x, B_wqkv, B_wo)
    return jnp.concatenate([a, b], axis=-1)
```

```python
import functools

import jax
import jax.numpy as jnp
from jax import lax
import jax.experimental.pallas as pl
import jax.experimental.pallas.tpu as pltpu

f32 = jnp.float32
bf16 = jnp.bfloat16
i32 = jnp.int32

S = 2048
D = 1024
NH = 32
HG = 4
MEM = 8
SEG = 32
NPAIR = S // (2 * SEG)
A_SCALE = 128 ** -0.5
B_SCALE = 32 ** -0.5
WIN, DIL = 8, 2
NT_J = 16
NG = 8
NSLOT = 3
PAD = 8
CHUNK_ROWS = 2048
MASKED = -1000000000.0
NEVER = -1e30

_NT = (((1,), (1,)), ((), ()))


def _as_bf16(x):
    return pltpu.bitcast(x, bf16)


def _as_i32(x):
    return pltpu.bitcast(x, i32)


def _lo_halves(a, b):
    return (a & 0xFFFF) | (b << 16)


def _hi_halves(a, b):
    return lax.shift_right_logical(a, 16) | (b & -65536)


def _a_masks():
    r = lax.broadcasted_iota(i32, (32, 128), 0)
    c = lax.broadcasted_iota(i32, (32, 128), 1)
    in_seg = (c < 32) | ((c >= 40) & (c < 48))
    ci = jnp.where(c < 32, c + 8, c - 40)
    vis_a = in_seg & ((r < 8) | (r >= ci))
    fill_a = jnp.where(in_seg, MASKED, NEVER).astype(f32)
    r = lax.broadcasted_iota(i32, (48, 128), 0)
    c = lax.broadcasted_iota(i32, (48, 128), 1)
    row_a = r < 8
    col_a = (c < 32) | ((c >= 40) & (c < 48))
    col_b = ((c >= 32) & (c < 40)) | ((c >= 48) & (c < 80))
    ri = jnp.where(r < 8, r + 32, jnp.where(r < 24, r, jnp.where(r < 32, r - 24, r - 8)))
    ci = jnp.where(c < 32, c + 8,
                   jnp.where(c < 40, c - 24,
                             jnp.where(c < 48, c - 40, jnp.where(c < 56, c - 48, c - 40))))
    in_seg = (row_a & col_a) | ((~row_a) & col_b)
    vis_b = in_seg & ((ri < 8) | (ri >= ci))
    fill_b = jnp.where(in_seg, MASKED, NEVER).astype(f32)
    return vis_a, fill_a, vis_b, fill_b


def _pad_keys(x):
    return jnp.concatenate([x, jnp.zeros((128 - x.shape[0], 128), bf16)], axis=0)


def _a_scores(q, k, vis, fill):
    s = lax.dot_general(q, _pad_keys(k), _NT, preferred_element_type=f32) * A_SCALE
    s = jnp.where(vis, s, fill)
    e = jnp.exp(s - jnp.max(s, axis=1, keepdims=True))
    return e.astype(bf16), 1.0 / jnp.sum(e, axis=1, keepdims=True)


def _a_values(e, inv, v):
    o = jnp.dot(e, _pad_keys(v), preferred_element_type=f32)
    return (o * inv).astype(bf16)


def _kernel(ax_hbm, mem0_ref, wq_hbm, wk_hbm, wv_hbm, awo_hbm, bx_hbm, bw_hbm, bwo_hbm,
            out_hbm,
            W, WO, XA, STG, XB, XP, WB, WT0, WT1, QKV0, QKV1, KVR0, KVR1, OB, WOB, OUTB,
            SQ, SK, SV, OA, MM, OUTA,
            sem_xb, sem_wb, sem_stg, sem_misc, sem_out):
    a_w = (wq_hbm, wk_hbm, wv_hbm)

    def slab_copy(src, col, dst, sem):
        return pltpu.make_async_copy(src.at[:, pl.ds(col, 128)], dst.bitcast(bf16), sem)

    def xb_copy(k):
        return slab_copy(bx_hbm, k * 128, XB.at[k], sem_xb.at[k])

    def wb_copies(g):
        return [slab_copy(bw_hbm, t * D + g * 128, WB.at[3 * g + t], sem_wb.at[g])
                for t in range(3)]

    def stg_copies(c):
        return [pltpu.make_async_copy(
            a_w[t].at[pl.ds(c * 2 * CHUNK_ROWS, 2 * CHUNK_ROWS), :],
            STG.at[c % NSLOT, t, pl.ds(PAD, CHUNK_ROWS), :].bitcast(bf16),
            sem_stg.at[c % NSLOT]) for t in range(3)]

    def wob_copies():
        return [slab_copy(bwo_hbm, c * 128, WOB.at[c], sem_misc.at[0]) for c in range(8)]

    def awo_copies():
        return [slab_copy(awo_hbm, c * 128, WO.at[c], sem_misc.at[1]) for c in range(8)]

    def xa_copies():
        return [slab_copy(ax_hbm, c * 128, XA.at[c], sem_misc.at[2]) for c in range(8)]

    def outb_copies():
        return [pltpu.make_async_copy(OUTB.at[c].bitcast(bf16),
                                      out_hbm.at[:, pl.ds(D + c * 128, 128)], sem_out.at[0])
                for c in range(8)]

    def outa_copy(p):
        rows = pl.ds(pl.multiple_of(p * 2 * SEG, 2 * SEG), 2 * SEG)
        return pltpu.make_async_copy(OUTA.at[rows, :], out_hbm.at[rows, pl.ds(0, D)],
                                     sem_out.at[1])

    def start(copies):
        for c in copies:
            c.start()

    def wait(copies):
        for c in copies:
            c.wait()

    def permute_x(k):
        for u in range(NT_J // 2):
            even = XB[k, pl.ds(u, 64, stride=16), :]
            odd = XB[k, pl.ds(u + 8, 64, stride=16), :]
            XP[2 * u, k] = _lo_halves(even, odd)
            XP[2 * u + 1, k] = _hi_halves(even, odd)

    def transpose_w(g, WT):
        for t in range(3):
            for k in range(8):
                tile = _as_bf16(WB[3 * g + t, k * 64:(k + 1) * 64, :])
                WT[k, t * 64:(t + 1) * 64, :] = _as_i32(tile.T)

    def project(WT, QKV, KVR):
        lhs = _as_bf16(jnp.concatenate([WT[k] for k in range(8)], axis=1))
        lane0 = lax.broadcasted_iota(i32, (128, 128), 1) == 0
        v_first = None
        for j in range(NT_J):
            x = _as_bf16(jnp.concatenate([XP[j, k] for k in range(8)], axis=1))
            y = lax.dot_general(lhs, x, _NT, preferred_element_type=f32)
            k, v = y[128:256], y[256:384]
            QKV[0, j] = y[0:128] * B_SCALE
            QKV[1, j] = k
            QKV[2, j] = v
            if j >= DIL:
                KVR[0, j - DIL] = pltpu.roll(k, 1, 1)
                KVR[1, j - DIL] = jnp.where(lane0, QKV[2, 0], pltpu.roll(v, 1, 1))

    def attend(g, QKV, KVR, tiles):
        lane0 = lax.broadcasted_iota(i32, (1, 128), 1) == 0
        for j in tiles:
            outs = []
            for hh in range(4):
                rows = slice(hh * 32, (hh + 1) * 32)

                def tap(t, w):
                    jj = j - DIL * w
                    return QKV[1 + t, jj, rows, :] if jj >= 0 else KVR[t, jj + NT_J - DIL, rows, :]

                q = QKV[0, j, rows, :]
                logits = []
                for w in range(WIN):
                    lg = jnp.sum(q * tap(0, w), axis=0, keepdims=True)
                    if j < DIL * w:
                        lg = jnp.where(lane0, MASKED, lg)
                    logits.append(lg)
                m = functools.reduce(jnp.maximum, logits)
                es = [jnp.exp(lg - m) for lg in logits]
                inv = 1.0 / functools.reduce(jnp.add, es)
                o = functools.reduce(jnp.add, [es[w] * tap(1, w) for w in range(WIN)])
                outs.append(o * inv)
            o_t = jnp.concatenate(outs, axis=0).astype(bf16)
            OB[j, g] = _as_i32(o_t.T)

    def project_out(u):
        lhs = _as_bf16(jnp.concatenate(
            [jnp.concatenate([OB[2 * u, g], OB[2 * u + 1, g]], axis=0) for g in range(NG)],
            axis=1))
        for c in range(8):
            y = jnp.dot(lhs, _as_bf16(WOB[c]), preferred_element_type=f32)
            word = pltpu.pack_elementwise([y[0:128], y[128:256]], packed_dtype=bf16)
            OUTB[c, pl.ds(u, 128, stride=8), :] = word.astype(i32)

    def relayout(c):
        sub = lax.broadcasted_iota(i32, (8, 128), 0)
        bits = [(sub & (1 << b)) != 0 for b in range(3)]
        for t in range(3):
            for b in range(CHUNK_ROWS // 256):
                base = PAD + 256 * b
                v = {i: STG[c % NSLOT, t, pl.ds(base + i, 8, stride=33), :]
                     for i in range(-7, 32)}
                for lo, s in ((-6, 0), (-4, 1), (0, 2)):
                    v = {i: jnp.where(bits[s], v[i - (1 << s)], v[i]) for i in range(lo, 32)}
                rows = pl.ds(c * 64 + 8 * b, 8)
                for i in range(16):
                    W[3 * (2 * i) + t, rows, :] = _lo_halves(v[i], v[16 + i])
                    W[3 * (2 * i + 1) + t, rows, :] = _hi_halves(v[i], v[16 + i])

    start([xb_copy(k) for k in range(8)])
    start(wb_copies(0))
    zeros = jnp.zeros((PAD, 128), i32)
    for slot in range(NSLOT):
        for t in range(3):
            STG[slot, t, 0:PAD, :] = zeros
            STG[slot, t, PAD + CHUNK_ROWS:, :] = zeros
    for k in range(8):
        xb_copy(k).wait()
        if k == 4:
            start(wb_copies(1))
        permute_x(k)
    for g in range(2, NG):
        start(wb_copies(g))
    for c in range(NSLOT):
        start(stg_copies(c))
    wait(wb_copies(0))
    transpose_w(0, WT0)

    bufs = ((WT0, QKV0, KVR0), (WT1, QKV1, KVR1))
    for g in range(NG):
        cur, other = bufs[g % 2], bufs[1 - g % 2]
        if g + 1 < NG:
            wait(wb_copies(g + 1))
        if g >= 1:
            wait(stg_copies(g - 1))
        if g >= 2 and g - 2 + NSLOT < NG:
            start(stg_copies(g - 2 + NSLOT))
        if g == 3:
            start(wob_copies())
        if g == 5:
            start(awo_copies())
        if g == 7:
            start(xa_copies())
        if g + 1 < NG:
            transpose_w(g + 1, other[0])
        project(*cur)
        if g >= 1:
            attend(g - 1, other[1], other[2], range(NT_J))
            relayout(g - 1)

    wait(wob_copies())
    wait(stg_copies(NG - 1))
    attend(NG - 1, QKV1, KVR1, range(0, 2))
    for u in range(NT_J // 2):
        if u + 1 < NT_J // 2:
            attend(NG - 1, QKV1, KVR1, range(2 * u + 2, 2 * u + 4))
        project_out(u)
    relayout(NG - 1)
    start(outb_copies())

    wait(awo_copies())
    wait(xa_copies())
    m0 = mem0_ref[...].astype(f32)
    for c in range(8):
        piece = m0[:, c * 128:(c + 1) * 128]
        MM[c] = _as_i32(jnp.concatenate([piece, piece], axis=0).astype(bf16))

    def step(lhs, rows, second, vis, fill):
        def proj(t, h):
            return jnp.dot(lhs, _as_bf16(W[3 * h + t]), preferred_element_type=f32)

        def out_part(h0, h1, c):
            o = _as_bf16(jnp.concatenate([OA[h, 0:rows // 2, :] for h in range(h0, h1)], axis=1))
            return jnp.dot(o, _as_bf16(WO[c, h0 * 64:h1 * 64, :]), preferred_element_type=f32)

        def finish(pending):
            for h, (e, inv, v) in pending.items():
                OA[h, 0:rows // 2, :] = _as_i32(_a_values(e, inv, v))

        pending = {}
        for g in range(NH // HG):
            heads = range(g * HG, (g + 1) * HG)
            q = {h: proj(0, h) for h in heads}
            k = {h: proj(1, h).astype(bf16) for h in heads}
            finish(pending)
            v = {h: proj(2, h).astype(bf16) for h in heads}
            pending = {}
            for h in heads:
                if not second:
                    SQ[h] = _as_i32(q[h][24:40].astype(bf16))
                    SK[h] = _as_i32(k[h])
                    SV[h] = _as_i32(v[h])
                    qq = jnp.concatenate([q[h][40:48], q[h][0:24]], axis=0).astype(bf16)
                    kk, vv = k[h], v[h]
                else:
                    qq = jnp.concatenate([q[h][8:16], q[h][0:8], q[h][16:32]], axis=0).astype(bf16)
                    qq = jnp.concatenate([_as_bf16(SQ[h]), qq], axis=0)
                    kk = jnp.concatenate([_as_bf16(SK[h]), k[h]], axis=0)
                    vv = jnp.concatenate([_as_bf16(SV[h]), v[h]], axis=0)
                e, inv = _a_scores(qq, kk, vis, fill)
                pending[h] = (e, inv, vv)
        first = [out_part(0, NH // 2, c) for c in range(4)]
        finish(pending)
        first += [out_part(0, NH // 2, c) for c in range(4, 8)]
        return [first[c] + out_part(NH // 2, NH, c) for c in range(8)]

    def pair(p, carry):
        vis_a, fill_a, vis_b, fill_b = _a_masks()
        low = lax.broadcasted_iota(i32, (8, 128), 0) < 4
        base = pl.multiple_of(p * SEG, SEG)
        orow = pl.multiple_of(p * 2 * SEG, 2 * SEG)
        mixed = [XA[c, pl.ds(base + 16, 8), :] for c in range(8)]
        lhs = _as_bf16(jnp.concatenate(
            [jnp.concatenate([XA[c, pl.ds(base, 16), :], jnp.where(low, mixed[c], MM[c])], axis=0)
             for c in range(8)], axis=1))
        ya = step(lhs, 32, False, vis_a, fill_a)
        pieces = []
        for c in range(8):
            mem = _as_i32(ya[c][0:16].astype(bf16))
            pieces.append(jnp.concatenate(
                [jnp.where(low, mem, mixed[c]), XA[c, pl.ds(base + 24, 8), :]], axis=0))
            OUTA[pl.ds(orow, 16), c * 128:(c + 1) * 128] = ya[c][8:24].astype(bf16)
        lhs = _as_bf16(jnp.concatenate(pieces, axis=1))
        zb = step(lhs, 48, True, vis_b, fill_b)
        for c in range(8):
            cols = slice(c * 128, (c + 1) * 128)
            MM[c] = _as_i32(zb[c][16:32].astype(bf16))
            OUTA[pl.ds(orow + 16, 16), cols] = jnp.concatenate(
                [ya[c][24:32], zb[c][0:8]], axis=0).astype(bf16)
            OUTA[pl.ds(orow + 32, 16), cols] = zb[c][8:24].astype(bf16)
            OUTA[pl.ds(orow + 48, 16), cols] = zb[c][32:48].astype(bf16)
        outa_copy(p).start()
        return carry

    lax.fori_loop(0, NPAIR, pair, 0)

    wait(outb_copies())
    for p in range(NPAIR):
        outa_copy(p).wait()


def _vmem(shape, dtype=i32):
    return pltpu.VMEM(shape, dtype)


@functools.partial(jax.jit, static_argnames=("A_seg_len",))
def pallas_concat_heads__memory_aug_recurrent_mem_tr__sliding_local_dilated__prompt_kernel(
    A_x: jax.Array,
    A_mem0: jax.Array,
    A_Wq: jax.Array,
    A_Wk: jax.Array,
    A_Wv: jax.Array,
    A_Wo: jax.Array,
    A_seg_len: int,
    B_x: jax.Array,
    B_wqkv: jax.Array,
    B_wo: jax.Array,
):
    assert A_seg_len == SEG and A_x.shape == (1, S, D) and A_mem0.shape == (1, MEM, D)
    assert A_Wq.shape == (D, NH, 128) and A_Wo.shape == (NH, 128, D)
    assert B_x.shape == (1, S, D) and B_wqkv.shape == (D, 3 * D) and B_wo.shape == (D, D)

    hbm = pl.BlockSpec(memory_space=pl.ANY)
    out = pl.pallas_call(
        _kernel,
        out_shape=jax.ShapeDtypeStruct((S, 2 * D), bf16),
        in_specs=[hbm, pl.BlockSpec(memory_space=pltpu.VMEM)] + [hbm] * 7,
        out_specs=hbm,
        scratch_shapes=[
            _vmem((3 * NH, 512, 128)),
            _vmem((8, 2048, 128)),
            _vmem((8, S // 2, 128)),
            _vmem((NSLOT, 3, CHUNK_ROWS + 2 * PAD, 128)),
            _vmem((8, S // 2, 128)),
            _vmem((NT_J, 8, 64, 128)),
            _vmem((3 * NG, 512, 128)),
            _vmem((8, 192, 128)),
            _vmem((8, 192, 128)),
            _vmem((3, NT_J, 128, 128), f32),
            _vmem((3, NT_J, 128, 128), f32),
            _vmem((2, NT_J - DIL, 128, 128), f32),
            _vmem((2, NT_J - DIL, 128, 128), f32),
            _vmem((NT_J, NG, 64, 128)),
            _vmem((8, 512, 128)),
            _vmem((8, S // 2, 128)),
            _vmem((NH, 8, 128)),
            _vmem((NH, 24, 128)),
            _vmem((NH, 24, 128)),
            _vmem((NH, 24, 128)),
            _vmem((8, 8, 128)),
            _vmem((S, D), bf16),
            pltpu.SemaphoreType.DMA((8,)),
            pltpu.SemaphoreType.DMA((NG,)),
            pltpu.SemaphoreType.DMA((NSLOT,)),
            pltpu.SemaphoreType.DMA((3,)),
            pltpu.SemaphoreType.DMA((2,)),
        ],
        compiler_params=pltpu.CompilerParams(vmem_limit_bytes=112 * 1024 * 1024),
    )(
        A_x.astype(bf16).reshape(S, D),
        A_mem0.astype(bf16).reshape(MEM, D),
        A_Wq.astype(bf16).reshape(D * NH, 128),
        A_Wk.astype(bf16).reshape(D * NH, 128),
        A_Wv.astype(bf16).reshape(D * NH, 128),
        A_Wo.astype(bf16).reshape(NH * 128, D),
        B_x.astype(bf16).reshape(S, D),
        B_wqkv.astype(bf16),
        B_wo.astype(bf16),
    )
    return out.reshape(1, S, 2 * D)
```

```python
import functools

import jax
import jax.numpy as jnp
from jax import lax
import jax.experimental.pallas as pl
import jax.experimental.pallas.tpu as pltpu

f32 = jnp.float32
bf16 = jnp.bfloat16
i32 = jnp.int32

S = 2048
D = 1024
NH = 32
HG = 4
MEM = 8
SEG = 32
NPAIR = S // (2 * SEG)
A_SCALE = 128 ** -0.5
B_SCALE = 32 ** -0.5
WIN, DIL = 8, 2
NT_J = 16
NG = 8
PAD = 8
CHUNK_ROWS = 2048
STG_ROWS = CHUNK_ROWS + 2 * PAD
HALO = NT_J - DIL
KV_TILES = HALO + NT_J
ACT_ROWS = (NT_J + 2 * KV_TILES) * 128
MASKED = -1000000000.0
NEVER = -1e30

_NT = (((1,), (1,)), ((), ()))


def _aligned(i, n):
    return i if isinstance(i, int) else pl.multiple_of(i, n)


def _as_bf16(x):
    return pltpu.bitcast(x, bf16)


def _as_i32(x):
    return pltpu.bitcast(x, i32)


def _lo_halves(a, b):
    return (a & 0xFFFF) | (b << 16)


def _hi_halves(a, b):
    return lax.shift_right_logical(a, 16) | (b & -65536)


def _a_masks():
    r = lax.broadcasted_iota(i32, (32, 128), 0)
    c = lax.broadcasted_iota(i32, (32, 128), 1)
    in_seg = (c < 32) | ((c >= 40) & (c < 48))
    ci = jnp.where(c < 32, c + 8, c - 40)
    vis_a = in_seg & ((r < 8) | (r >= ci))
    fill_a = jnp.where(in_seg, MASKED, NEVER).astype(f32)
    r = lax.broadcasted_iota(i32, (48, 128), 0)
    c = lax.broadcasted_iota(i32, (48, 128), 1)
    row_a = r < 8
    col_a = (c < 32) | ((c >= 40) & (c < 48))
    col_b = ((c >= 32) & (c < 40)) | ((c >= 48) & (c < 80))
    ri = jnp.where(r < 8, r + 32, jnp.where(r < 24, r, jnp.where(r < 32, r - 24, r - 8)))
    ci = jnp.where(c < 32, c + 8,
                   jnp.where(c < 40, c - 24,
                             jnp.where(c < 48, c - 40, jnp.where(c < 56, c - 48, c - 40))))
    in_seg = (row_a & col_a) | ((~row_a) & col_b)
    vis_b = in_seg & ((ri < 8) | (ri >= ci))
    fill_b = jnp.where(in_seg, MASKED, NEVER).astype(f32)
    return vis_a, fill_a, vis_b, fill_b


def _pad_keys(x):
    return jnp.concatenate([x, jnp.zeros((128 - x.shape[0], 128), bf16)], axis=0)


def _a_probs(q, k, vis, fill):
    s = lax.dot_general(q, _pad_keys(k), _NT, preferred_element_type=f32) * A_SCALE
    s = jnp.where(vis, s, fill)
    e = jnp.exp(s - jnp.max(s, axis=1, keepdims=True))
    return (e * (1.0 / jnp.sum(e, axis=1, keepdims=True))).astype(bf16)


def _a_values(p, v):
    return jnp.dot(p, _pad_keys(v), preferred_element_type=f32).astype(bf16)


def _kernel(ax_hbm, mem0_ref, wq_hbm, wk_hbm, wv_hbm, awo_hbm, bx_hbm, bw_hbm, bwo_hbm,
            out_hbm,
            W, WO, XA, STG, XB, XP, WB, WT0, WT1, ACT0, ACT1, OB, WOB, OUTB,
            SQ, SK, SV, OA, PART, MM, OUTA, ZERO,
            sem_xb, sem_wb, sem_misc, sem_out):
    a_w = (wq_hbm, wk_hbm, wv_hbm)

    def slab_copy(src, col, dst, sem):
        return pltpu.make_async_copy(src.at[:, pl.ds(_aligned(col, 128), 128)],
                                     dst.bitcast(bf16), sem)

    def xb_copy(k):
        return slab_copy(bx_hbm, k * 128, XB.at[k], sem_xb.at[k])

    def wb_copies(g):
        return [slab_copy(bw_hbm, t * D + g * 128, WB.at[3 * g + t], sem_wb.at[g])
                for t in range(3)]

    def stg_copies(c):
        return [pltpu.make_async_copy(
            a_w[t].at[pl.ds(c * 2 * CHUNK_ROWS, 2 * CHUNK_ROWS), :],
            STG.at[pl.ds((c * 3 + t) * STG_ROWS + PAD, CHUNK_ROWS), :].bitcast(bf16),
            sem_misc.at[3]) for t in range(3)]

    def wob_copies():
        return [slab_copy(bwo_hbm, c * 128, WOB.at[c], sem_misc.at[0]) for c in range(8)]

    def awo_copies():
        return [slab_copy(awo_hbm, c * 128, WO.at[c], sem_misc.at[1]) for c in range(8)]

    def xa_copies():
        return [slab_copy(ax_hbm, c * 128, XA.at[c], sem_misc.at[2]) for c in range(8)]

    def outb_copies():
        return [pltpu.make_async_copy(OUTB.at[c].bitcast(bf16),
                                      out_hbm.at[:, pl.ds(D + c * 128, 128)], sem_out.at[0])
                for c in range(8)]

    def outa_copy(p):
        rows = pl.ds(pl.multiple_of(p * 2 * SEG, 2 * SEG), 2 * SEG)
        return pltpu.make_async_copy(OUTA.at[rows, :], out_hbm.at[rows, pl.ds(0, D)],
                                     sem_out.at[1])

    def start(copies):
        for c in copies:
            c.start()

    def wait(copies):
        for c in copies:
            c.wait()

    def permute_x(k):
        for u in range(NT_J // 2):
            even = XB[k, pl.ds(u, 64, stride=16), :]
            odd = XB[k, pl.ds(u + 8, 64, stride=16), :]
            XP[2 * u, k] = _lo_halves(even, odd)
            XP[2 * u + 1, k] = _hi_halves(even, odd)

    def transpose_w(g, WT, items):
        for t, k in items:
            tile = _as_bf16(WB[3 * g + t, k * 64:(k + 1) * 64, :])
            WT[k, t * 64:(t + 1) * 64, :] = _as_i32(tile.T)

    def after(y):
        return _as_i32(y[0:8])[0, 0] * ZERO[0]

    def act_rows(t, j, row=0, n=128, start=0):
        tile = j if t == 0 else NT_J + (t - 1) * KV_TILES + HALO + j
        return pl.ds(_aligned(start + tile * 128 + row, 8), n)

    def project(WT, ACT, j, t):
        lhs = _as_bf16(jnp.concatenate([WT[k, t * 64:(t + 1) * 64, :] for k in range(8)], axis=1))
        x = _as_bf16(jnp.concatenate([XP[j, k] for k in range(8)], axis=1))
        y = lax.dot_general(lhs, x, _NT, preferred_element_type=f32)
        if t == 0:
            y = y * B_SCALE
        ACT[act_rows(t, j), :] = y
        if t > 0 and j >= DIL:
            y = pltpu.roll(y, 1, 1)
            if t == 2:
                lane0 = lax.broadcasted_iota(i32, (128, 128), 1) == 0
                y = jnp.where(lane0, ACT[act_rows(t, 0), :], y)
            ACT[act_rows(t, j - NT_J), :] = y
        return after(y)

    def attend_head(ACT, j, hh, start):
        def load(t, jj):
            return ACT[act_rows(t, jj, hh * 32, 32, start), :]

        q = load(0, j)
        logits = []
        for w in range(WIN):
            lg = jnp.sum(q * load(1, j - DIL * w), axis=0, keepdims=True)
            if j < DIL * w:
                lg = jnp.where(lax.broadcasted_iota(i32, (1, 128), 1) == 0, MASKED, lg)
            logits.append(lg)
        m = functools.reduce(jnp.maximum, logits)
        es = [jnp.exp(lg - m) for lg in logits]
        inv = 1.0 / functools.reduce(jnp.add, es)
        o = functools.reduce(jnp.add, [es[w] * load(2, j - DIL * w) for w in range(WIN)])
        return (o * inv).astype(bf16)

    def store_heads(g, j, heads):
        OB[j, g] = _as_i32(jnp.concatenate(heads, axis=0).T)

    def project_out(j, c):
        lhs = _as_bf16(jnp.concatenate([OB[j, g] for g in range(NG)], axis=1))
        return jnp.dot(lhs, _as_bf16(WOB[c]), preferred_element_type=f32)

    def relayout(c, items, start):
        sub = lax.broadcasted_iota(i32, (8, 128), 0)
        bits = [(sub & (1 << b)) != 0 for b in range(3)]
        for t, b in items:
            base = start + (c * 3 + t) * STG_ROWS + PAD + 256 * b
            rows = pl.ds(c * 64 + 8 * b, 8)
            v = [{}, {}, {}, {}]
            for i in range(-7, 32):
                v[0][i] = STG[pl.ds(base + i, 8, stride=33), :]
                for s in range(3):
                    if i - (1 << s) in v[s]:
                        v[s + 1][i] = jnp.where(bits[s], v[s][i - (1 << s)], v[s][i])
                if i >= 16:
                    even, odd = v[3][i - 16], v[3][i]
                    W[3 * (2 * (i - 16)) + t, rows, :] = _lo_halves(even, odd)
                    W[3 * (2 * (i - 16) + 1) + t, rows, :] = _hi_halves(even, odd)

    items = [(t, k) for t in range(3) for k in range(8)]

    def share(n, j):
        return items[len(items) * j // n:len(items) * (j + 1) // n]

    start([xb_copy(k) for k in range(8)])
    start(wb_copies(0))
    zeros = jnp.zeros((PAD, 128), i32)
    for slot in range(NG):
        for t in range(3):
            row = (slot * 3 + t) * STG_ROWS
            STG[row:row + PAD, :] = zeros
            STG[row + PAD + CHUNK_ROWS:row + STG_ROWS, :] = zeros
    ZERO[0] = 0
    for k in range(8):
        xb_copy(k).wait()
        if k == 4:
            start(wb_copies(1))
        permute_x(k)
    for g in range(2, NG):
        start(wb_copies(g))
    wait(wb_copies(0))
    transpose_w(0, WT0, items)
    wait(wb_copies(1))
    for c in range(NG):
        start(stg_copies(c))

    def group(g, parity, first=False, last=False):
        wt, wt_next = (WT0, WT1)[parity], (WT0, WT1)[1 - parity]
        act, act_prev = (ACT0, ACT1)[parity], (ACT0, ACT1)[1 - parity]
        zero = 0
        for j in range(NT_J):
            heads = []
            for t in range(3):
                zero, prev = project(wt, act, j, t), zero
                if not last and t == 0:
                    transpose_w(g + 1, wt_next, share(NT_J, j))
                if not first:
                    heads += [attend_head(act_prev, j, hh, prev)
                              for hh in ((0,), (1, 2), (3,))[t]]
            if not first:
                store_heads(g - 1, j, heads)

    group(0, 0, first=True)
    for g in range(2, NG):
        wait(wb_copies(g))
    start(wob_copies())
    start(awo_copies())
    start(xa_copies())

    def two_groups(i, carry):
        group(2 * i + 1, 1)
        group(2 * i + 2, 0)
        return carry

    lax.fori_loop(0, (NG - 2) // 2, two_groups, 0)
    group(NG - 1, 1, last=True)

    wait(wob_copies())
    for c in range(NG):
        wait(stg_copies(c))
    for j in range(2):
        store_heads(NG - 1, j, [attend_head(ACT1, j, hh, 0) for hh in range(4)])
    zero = 0
    for u in range(NT_J // 2):
        heads = []
        for c in range(8):
            blocks = share(8, c)
            y0 = project_out(2 * u, c)
            relayout(u, blocks[:2], zero)
            y1 = project_out(2 * u + 1, c)
            mid = after(y0)
            relayout(u, blocks[2:], mid)
            if u + 1 < NT_J // 2:
                j = 2 * u + 2 + c // 4
                heads.append(attend_head(ACT1, j, c % 4, mid))
                if c % 4 == 3:
                    store_heads(NG - 1, j, heads)
                    heads = []
            zero = after(y1)
            word = pltpu.pack_elementwise([y0, y1], packed_dtype=bf16)
            OUTB[c, pl.ds(u, 128, stride=8), :] = word.astype(i32)
    start(outb_copies())

    wait(awo_copies())
    wait(xa_copies())
    m0 = mem0_ref[...].astype(f32)
    for c in range(8):
        piece = m0[:, c * 128:(c + 1) * 128]
        MM[c] = _as_i32(jnp.concatenate([piece, piece], axis=0).astype(bf16))

    def step(lhs, rows, second, vis, fill):
        def proj(t, h):
            return jnp.dot(lhs, _as_bf16(W[3 * h + t]), preferred_element_type=f32)

        def out_part(h0, h1, c):
            o = _as_bf16(jnp.concatenate([OA[h, 0:rows // 2, :] for h in range(h0, h1)], axis=1))
            return jnp.dot(o, _as_bf16(WO[c, h0 * 64:h1 * 64, :]), preferred_element_type=f32)

        def finish(pending):
            for h, (prob, v) in pending.items():
                OA[h, 0:rows // 2, :] = _as_i32(_a_values(prob, v))

        pending = {}
        for g in range(NH // HG):
            heads = range(g * HG, (g + 1) * HG)
            q = {h: proj(0, h) for h in heads}
            k = {h: proj(1, h).astype(bf16) for h in heads}
            finish(pending)
            v = {h: proj(2, h).astype(bf16) for h in heads}
            pending = {}
            for h in heads:
                if not second:
                    SQ[h] = _as_i32(q[h][24:40].astype(bf16))
                    SK[h] = _as_i32(k[h])
                    SV[h] = _as_i32(v[h])
                    qq = jnp.concatenate([q[h][40:48], q[h][0:24]], axis=0).astype(bf16)
                    kk, vv = k[h], v[h]
                else:
                    qq = jnp.concatenate([q[h][8:16], q[h][0:8], q[h][16:32]], axis=0).astype(bf16)
                    qq = jnp.concatenate([_as_bf16(SQ[h]), qq], axis=0)
                    kk = jnp.concatenate([_as_bf16(SK[h]), k[h]], axis=0)
                    vv = jnp.concatenate([_as_bf16(SV[h]), v[h]], axis=0)
                pending[h] = (_a_probs(qq, kk, vis, fill), vv)
        for c in range(4):
            PART[c, 0:rows, :] = out_part(0, NH // 2, c)
        finish(pending)
        for c in range(4, 8):
            PART[c, 0:rows, :] = out_part(0, NH // 2, c)
        return [PART[c, 0:rows, :] + out_part(NH // 2, NH, c) for c in range(8)]

    def pair(p, carry):
        vis_a, fill_a, vis_b, fill_b = _a_masks()
        low = lax.broadcasted_iota(i32, (8, 128), 0) < 4
        base = pl.multiple_of(p * SEG, SEG)
        orow = pl.multiple_of(p * 2 * SEG, 2 * SEG)
        mixed = [XA[c, pl.ds(base + 16, 8), :] for c in range(8)]
        lhs = _as_bf16(jnp.concatenate(
            [jnp.concatenate([XA[c, pl.ds(base, 16), :], jnp.where(low, mixed[c], MM[c])], axis=0)
             for c in range(8)], axis=1))
        ya = step(lhs, 32, False, vis_a, fill_a)
        pieces = []
        for c in range(8):
            mem = _as_i32(ya[c][0:16].astype(bf16))
            pieces.append(jnp.concatenate(
                [jnp.where(low, mem, mixed[c]), XA[c, pl.ds(base + 24, 8), :]], axis=0))
            OUTA[pl.ds(orow, 16), c * 128:(c + 1) * 128] = ya[c][8:24].astype(bf16)
        lhs = _as_bf16(jnp.concatenate(pieces, axis=1))
        zb = step(lhs, 48, True, vis_b, fill_b)
        for c in range(8):
            cols = slice(c * 128, (c + 1) * 128)
            MM[c] = _as_i32(zb[c][16:32].astype(bf16))
            OUTA[pl.ds(orow + 16, 16), cols] = jnp.concatenate(
                [ya[c][24:32], zb[c][0:8]], axis=0).astype(bf16)
            OUTA[pl.ds(orow + 32, 16), cols] = zb[c][8:24].astype(bf16)
            OUTA[pl.ds(orow + 48, 16), cols] = zb[c][32:48].astype(bf16)
        outa_copy(p).start()
        return carry

    lax.fori_loop(0, NPAIR, pair, 0)

    wait(outb_copies())
    for p in range(NPAIR):
        outa_copy(p).wait()


def _vmem(shape, dtype=i32):
    return pltpu.VMEM(shape, dtype)


@functools.partial(jax.jit, static_argnames=("A_seg_len",))
def pallas_concat_heads__memory_aug_recurrent_mem_tr__sliding_local_dilated__prompt_kernel(
    A_x: jax.Array,
    A_mem0: jax.Array,
    A_Wq: jax.Array,
    A_Wk: jax.Array,
    A_Wv: jax.Array,
    A_Wo: jax.Array,
    A_seg_len: int,
    B_x: jax.Array,
    B_wqkv: jax.Array,
    B_wo: jax.Array,
):
    assert A_seg_len == SEG and A_x.shape == (1, S, D) and A_mem0.shape == (1, MEM, D)
    assert A_Wq.shape == (D, NH, 128) and A_Wo.shape == (NH, 128, D)
    assert B_x.shape == (1, S, D) and B_wqkv.shape == (D, 3 * D) and B_wo.shape == (D, D)

    hbm = pl.BlockSpec(memory_space=pl.ANY)
    out = pl.pallas_call(
        _kernel,
        out_shape=jax.ShapeDtypeStruct((S, 2 * D), bf16),
        in_specs=[hbm, pl.BlockSpec(memory_space=pltpu.VMEM)] + [hbm] * 7,
        out_specs=hbm,
        scratch_shapes=[
            _vmem((3 * NH, 512, 128)),
            _vmem((8, 2048, 128)),
            _vmem((8, S // 2, 128)),
            _vmem((NG * 3 * STG_ROWS, 128)),
            _vmem((8, S // 2, 128)),
            _vmem((NT_J, 8, 64, 128)),
            _vmem((3 * NG, 512, 128)),
            _vmem((8, 192, 128)),
            _vmem((8, 192, 128)),
            _vmem((ACT_ROWS, 128), f32),
            _vmem((ACT_ROWS, 128), f32),
            _vmem((NT_J, NG, 64, 128)),
            _vmem((8, 512, 128)),
            _vmem((8, S // 2, 128)),
            _vmem((NH, 8, 128)),
            _vmem((NH, 24, 128)),
            _vmem((NH, 24, 128)),
            _vmem((NH, 24, 128)),
            _vmem((8, 48, 128), f32),
            _vmem((8, 8, 128)),
            _vmem((S, D), bf16),
            pltpu.SMEM((1,), i32),
            pltpu.SemaphoreType.DMA((8,)),
            pltpu.SemaphoreType.DMA((NG,)),
            pltpu.SemaphoreType.DMA((4,)),
            pltpu.SemaphoreType.DMA((2,)),
        ],
        compiler_params=pltpu.CompilerParams(vmem_limit_bytes=112 * 1024 * 1024),
    )(
        A_x.astype(bf16).reshape(S, D),
        A_mem0.astype(bf16).reshape(MEM, D),
        A_Wq.astype(bf16).reshape(D * NH, 128),
        A_Wk.astype(bf16).reshape(D * NH, 128),
        A_Wv.astype(bf16).reshape(D * NH, 128),
        A_Wo.astype(bf16).reshape(NH * 128, D),
        B_x.astype(bf16).reshape(S, D),
        B_wqkv.astype(bf16),
        B_wo.astype(bf16),
    )
    return out.reshape(1, S, 2 * D)
```

```python
import functools

import jax
import jax.numpy as jnp
from jax import lax
import jax.experimental.pallas as pl
import jax.experimental.pallas.tpu as pltpu

f32 = jnp.float32
bf16 = jnp.bfloat16
i32 = jnp.int32

S = 2048
D = 1024
NH = 32
HG = 4
MEM = 8
SEG = 32
NPAIR = S // (2 * SEG)
A_SCALE = 128 ** -0.5
LOG2E = 1.4426950408889634
B_SCALE = 32 ** -0.5 * LOG2E
WIN, DIL = 8, 2
NT_J = 16
NG = 8
HALO = WIN - 1
KV_TILES = HALO + NT_J
ACT_TILES = NT_J + 2 * KV_TILES + 1
MASKED = -1000000000.0
NEVER = -1e30

_NT = (((1,), (1,)), ((), ()))


def _aligned(i, n):
    return i if isinstance(i, int) else pl.multiple_of(i, n)


def _as_bf16(x):
    return pltpu.bitcast(x, bf16)


def _as_i32(x):
    return pltpu.bitcast(x, i32)


def _interleave(a, b):
    def high(x):
        return pltpu.unpack_elementwise(x, index=1, packed_dtype=jnp.int16, unpacked_dtype=i32)

    def pack(x, y):
        return pltpu.pack_elementwise([x, y], packed_dtype=jnp.int16).astype(i32)

    return pack(a, b), pack(high(a), high(b))


def _a_masks():
    r = lax.broadcasted_iota(i32, (32, 128), 0)
    c = lax.broadcasted_iota(i32, (32, 128), 1)
    in_seg = (c < 32) | ((c >= 40) & (c < 48))
    ci = jnp.where(c < 32, c + 8, c - 40)
    vis_a = in_seg & ((r < 8) | (r >= ci))
    fill_a = jnp.where(in_seg, MASKED, NEVER).astype(f32)
    r = lax.broadcasted_iota(i32, (48, 128), 0)
    c = lax.broadcasted_iota(i32, (48, 128), 1)
    row_a = r < 8
    col_a = (c < 32) | ((c >= 40) & (c < 48))
    col_b = ((c >= 32) & (c < 40)) | ((c >= 48) & (c < 80))
    ri = jnp.where(r < 8, r + 32, jnp.where(r < 24, r, jnp.where(r < 32, r - 24, r - 8)))
    ci = jnp.where(c < 32, c + 8,
                   jnp.where(c < 40, c - 24,
                             jnp.where(c < 48, c - 40, jnp.where(c < 56, c - 48, c - 40))))
    in_seg = (row_a & col_a) | ((~row_a) & col_b)
    vis_b = in_seg & ((ri < 8) | (ri >= ci))
    fill_b = jnp.where(in_seg, MASKED, NEVER).astype(f32)
    return vis_a, fill_a, vis_b, fill_b


def _pad_keys(x):
    return jnp.concatenate([x, jnp.zeros((128 - x.shape[0], 128), bf16)], axis=0)


def _a_probs(q, k, vis, fill):
    s = lax.dot_general(q, _pad_keys(k), _NT, preferred_element_type=f32) * A_SCALE
    s = jnp.where(vis, s, fill)
    e = jnp.exp(s - jnp.max(s, axis=1, keepdims=True))
    return (e * (1.0 / jnp.sum(e, axis=1, keepdims=True))).astype(bf16)


def _a_values(p, v):
    return jnp.dot(p, _pad_keys(v), preferred_element_type=f32).astype(bf16)


def _kernel(ax_hbm, mem0_ref, wq_hbm, wk_hbm, wv_hbm, awo_hbm, bx_hbm, bw_hbm, bwo_hbm,
            out_hbm,
            W, WO, XA, XP, WB, WT0, WT1, ACT0, ACT1, OB, WOB, OUTB,
            SQ, SK, SV, OA, PART, MM, OUTA, ZERO,
            sem_xp, sem_wb, sem_misc, sem_out):
    def slab_copy(src, col, dst, sem):
        return pltpu.make_async_copy(src.at[:, pl.ds(_aligned(col, 128), 128)],
                                     dst.bitcast(bf16), sem)

    def xp_copy(j):
        return pltpu.make_async_copy(bx_hbm.bitcast(i32).at[:, j, :], XP.at[j], sem_xp.at[j])

    def wb_copies(g):
        return [slab_copy(bw_hbm, t * D + g * 128, WB.at[3 * g + t], sem_wb.at[g])
                for t in range(3)]

    def w_copies(t):
        src = (wq_hbm, wk_hbm, wv_hbm)[t].bitcast(i32)
        return [pltpu.make_async_copy(src.at[:, 16 * e + i, :], W.at[3 * (2 * i + e) + t],
                                      sem_misc.at[3])
                for i in range(NH // 2) for e in range(2)]

    def wob_copies():
        return [slab_copy(bwo_hbm, c * 128, WOB.at[c], sem_misc.at[0]) for c in range(8)]

    def awo_copies():
        return [slab_copy(awo_hbm, c * 128, WO.at[c], sem_misc.at[1]) for c in range(8)]

    def xa_copies():
        return [slab_copy(ax_hbm, c * 128, XA.at[c], sem_misc.at[2]) for c in range(8)]

    def outb_copies():
        return [pltpu.make_async_copy(OUTB.at[j], out_hbm.bitcast(i32).at[:, j, pl.ds(D, D)],
                                      sem_out.at[0]) for j in range(NT_J)]

    def outa_copy(p):
        segs = pl.ds(2 * p, 2)
        return pltpu.make_async_copy(OUTA.at[segs], out_hbm.at[segs, :, pl.ds(0, D)],
                                     sem_out.at[1])

    def start(copies):
        for c in copies:
            c.start()

    def wait(copies):
        for c in copies:
            c.wait()

    def transpose_w(g, WT, items):
        for t, k in items:
            tile = _as_bf16(WB[3 * g + t, k * 64:(k + 1) * 64, :])
            WT[k, t * 64:(t + 1) * 64, :] = _as_i32(tile.T)

    def after(x, token):
        if token is None:
            return x
        token = pltpu.bitcast(jnp.concatenate([token] * (x.shape[0] // 8), axis=0), x.dtype)
        return jnp.where(jnp.full(x.shape, ZERO[0], i32) == 0, x, token)

    def act_tile(t, j):
        return j if t == 0 else NT_J + (t - 1) * KV_TILES + HALO + j

    def project(WT, ACT, j, t):
        lhs = _as_bf16(jnp.concatenate([WT[k, t * 64:(t + 1) * 64, :] for k in range(8)], axis=1))
        y = lax.dot_general(lhs, _as_bf16(XP[j]), _NT, preferred_element_type=f32)
        if t == 0:
            y = y * B_SCALE
        ACT[act_tile(t, j)] = y
        lane = lax.broadcasted_iota(i32, (128, 128), 1)
        if t == 2 and j == 0:
            ACT[ACT_TILES - 1] = jnp.where(lane == 0, y, pltpu.roll(y, 1, 1))
        if t > 0 and j >= NT_J - HALO:
            shifted = pltpu.roll(y, 2, 1)
            if t == 2:
                shifted = jnp.where(lane < 2, ACT[ACT_TILES - 1], shifted)
            ACT[act_tile(t, j - NT_J)] = shifted
        return y[0:8], y[120:128]

    def attend_head(ACT, j, hh, token):
        def load(t, jj):
            return ACT[act_tile(t, jj), hh * 32:(hh + 1) * 32, :]

        q = after(load(0, j), token)
        logits = []
        for w in range(WIN):
            lg = jnp.sum(q * load(1, j - w), axis=0, keepdims=True)
            if j < w:
                lg = jnp.where(lax.broadcasted_iota(i32, (1, 128), 1) < 2, MASKED * LOG2E, lg)
            logits.append(lg)
        m = functools.reduce(jnp.maximum, logits)
        es = [jnp.exp2(lg - m) for lg in logits]
        inv = 1.0 / functools.reduce(jnp.add, es)
        o = functools.reduce(jnp.add, [es[w] * load(2, j - w) for w in range(WIN)])
        return (o * inv).astype(bf16)

    def store_heads(g, j, heads):
        OB[j, g] = _as_i32(jnp.concatenate(heads, axis=0).T)

    def project_out(j, c):
        lhs = _as_bf16(jnp.concatenate([OB[j, g] for g in range(NG)], axis=1))
        y = jnp.dot(lhs, _as_bf16(WOB[c]), preferred_element_type=f32)
        OUTB[j, :, c * 128:(c + 1) * 128] = _as_i32(y.astype(bf16))
        return y[0:8], y[120:128]

    def split_heads(item, token):
        slab, part = divmod(item, 8)
        t, i = divmod(slab, NH // 2)
        rows = slice(part * 64, (part + 1) * 64)
        even, odd = 3 * (2 * i) + t, 3 * (2 * i + 1) + t
        W[even, rows, :], W[odd, rows, :] = _interleave(after(W[even, rows, :], token),
                                                        after(W[odd, rows, :], token))

    w_tiles = [(t, k) for t in range(3) for k in range(8)]

    def share(items, n, j):
        return items[len(items) * j // n:len(items) * (j + 1) // n]

    def xp_copies(lo, hi):
        return [xp_copy(j) for j in range(lo, hi)]

    start(wb_copies(0))
    start(xp_copies(0, 3))
    ZERO[0] = 0
    wait(wb_copies(0))
    start(xp_copies(3, 7))
    transpose_w(0, WT0, w_tiles)

    def first_group_dma(j):
        if j == 0:
            wait(xp_copies(0, 1))
        elif j == 1:
            wait(xp_copies(1, 3))
            start(xp_copies(7, NT_J))
        elif j == 3:
            wait(xp_copies(3, 7))
            start(wb_copies(1))
        elif j == 7:
            wait(xp_copies(7, NT_J))
            wait(wb_copies(1))
            start(wb_copies(2) + wb_copies(3))

    def group(g, parity, first=False, last=False, dma=None):
        wt, wt_next = (WT0, WT1)[parity], (WT0, WT1)[1 - parity]
        act, act_prev = (ACT0, ACT1)[parity], (ACT0, ACT1)[1 - parity]
        tokens = (None, None)
        for j in range(NT_J):
            if dma is not None:
                dma(j)
            heads = []
            for t in range(3):
                tokens, prev = project(wt, act, j, t), tokens
                if t == 0 and first and j >= 7:
                    transpose_w(1, wt_next, share(w_tiles, NT_J - 7, j - 7))
                if t == 0 and not first and not last:
                    transpose_w(g + 1, wt_next, share(w_tiles, NT_J, j))
                if not first:
                    heads += [attend_head(act_prev, j, hh, prev[when]) for hh, when in
                              (((0, 1),), ((1, 0),), ((2, 0), (3, 1)))[t]]
            if not first:
                store_heads(g - 1, j, heads)

    group(0, 0, first=True, dma=first_group_dma)

    def two_groups(i, carry):
        wait(wb_copies(2 * i + 2) + wb_copies(2 * i + 3))

        later = [c for g in range(4, NG) for c in wb_copies(g)] + wob_copies()
        for t, others in enumerate((later, awo_copies(), xa_copies())):
            pl.when(i == t)(functools.partial(start, others + w_copies(t)))
        group(2 * i + 1, 1)
        group(2 * i + 2, 0)
        return carry

    lax.fori_loop(0, (NG - 2) // 2, two_groups, 0)
    group(NG - 1, 1, last=True)

    wait(wob_copies())
    wait(w_copies(0) + w_copies(1) + w_copies(2))
    store_heads(NG - 1, 0, [attend_head(ACT1, 0, hh, None) for hh in range(4)])
    tokens = (None, None)
    w_items = list(range(3 * (NH // 2) * 8))
    for j in range(NT_J):
        heads = []
        for c in range(8):
            tokens, prev = project_out(j, c), tokens
            if j + 1 < NT_J and c % 2 == 0:
                heads.append(attend_head(ACT1, j + 1, c // 2, prev[0]))
            for item in share(w_items, NT_J * 8, j * 8 + c):
                split_heads(item, prev[1])
        if heads:
            store_heads(NG - 1, j + 1, heads)
    start(outb_copies())

    wait(awo_copies())
    wait(xa_copies())
    m0 = mem0_ref[...].astype(f32)
    for c in range(8):
        piece = m0[:, c * 128:(c + 1) * 128]
        MM[c] = _as_i32(jnp.concatenate([piece, piece], axis=0).astype(bf16))

    def step(lhs, rows, second, vis, fill):
        def proj(t, h):
            return jnp.dot(lhs, _as_bf16(W[3 * h + t]), preferred_element_type=f32)

        def out_part(h0, h1, c):
            o = _as_bf16(jnp.concatenate([OA[h, 0:rows // 2, :] for h in range(h0, h1)], axis=1))
            return jnp.dot(o, _as_bf16(WO[c, h0 * 64:h1 * 64, :]), preferred_element_type=f32)

        def finish(pending):
            for h, (prob, v) in pending.items():
                OA[h, 0:rows // 2, :] = _as_i32(_a_values(prob, v))

        pending = {}
        for g in range(NH // HG):
            heads = range(g * HG, (g + 1) * HG)
            q = {h: proj(0, h) for h in heads}
            k = {h: proj(1, h).astype(bf16) for h in heads}
            finish(pending)
            v = {h: proj(2, h).astype(bf16) for h in heads}
            pending = {}
            for h in heads:
                if not second:
                    SQ[h] = _as_i32(q[h][24:40].astype(bf16))
                    SK[h] = _as_i32(k[h])
                    SV[h] = _as_i32(v[h])
                    qq = jnp.concatenate([q[h][40:48], q[h][0:24]], axis=0).astype(bf16)
                    kk, vv = k[h], v[h]
                else:
                    qq = jnp.concatenate([q[h][8:16], q[h][0:8], q[h][16:32]], axis=0).astype(bf16)
                    qq = jnp.concatenate([_as_bf16(SQ[h]), qq], axis=0)
                    kk = jnp.concatenate([_as_bf16(SK[h]), k[h]], axis=0)
                    vv = jnp.concatenate([_as_bf16(SV[h]), v[h]], axis=0)
                pending[h] = (_a_probs(qq, kk, vis, fill), vv)
        for c in range(4):
            PART[c, 0:rows, :] = out_part(0, NH // 2, c)
        finish(pending)
        for c in range(4, 8):
            PART[c, 0:rows, :] = out_part(0, NH // 2, c)
        return [PART[c, 0:rows, :] + out_part(NH // 2, NH, c) for c in range(8)]

    def pair(p, carry):
        vis_a, fill_a, vis_b, fill_b = _a_masks()
        low = lax.broadcasted_iota(i32, (8, 128), 0) < 4
        base = pl.multiple_of(p * SEG, SEG)
        mixed = [XA[c, pl.ds(base + 16, 8), :] for c in range(8)]
        lhs = _as_bf16(jnp.concatenate(
            [jnp.concatenate([XA[c, pl.ds(base, 16), :], jnp.where(low, mixed[c], MM[c])], axis=0)
             for c in range(8)], axis=1))
        ya = step(lhs, 32, False, vis_a, fill_a)
        pieces = []
        for c in range(8):
            mem = _as_i32(ya[c][0:16].astype(bf16))
            pieces.append(jnp.concatenate(
                [jnp.where(low, mem, mixed[c]), XA[c, pl.ds(base + 24, 8), :]], axis=0))
            OUTA[2 * p, 0:16, c * 128:(c + 1) * 128] = ya[c][8:24].astype(bf16)
        lhs = _as_bf16(jnp.concatenate(pieces, axis=1))
        zb = step(lhs, 48, True, vis_b, fill_b)
        for c in range(8):
            cols = slice(c * 128, (c + 1) * 128)
            MM[c] = _as_i32(zb[c][16:32].astype(bf16))
            OUTA[2 * p, 16:32, cols] = jnp.concatenate(
                [ya[c][24:32], zb[c][0:8]], axis=0).astype(bf16)
            OUTA[2 * p + 1, 0:16, cols] = zb[c][8:24].astype(bf16)
            OUTA[2 * p + 1, 16:32, cols] = zb[c][32:48].astype(bf16)
        outa_copy(p).start()
        return carry

    lax.fori_loop(0, NPAIR, pair, 0)

    wait(outb_copies())
    for p in range(NPAIR):
        outa_copy(p).wait()


def _vmem(shape, dtype=i32):
    return pltpu.VMEM(shape, dtype)


@functools.partial(jax.jit, static_argnames=("A_seg_len",))
def pallas_concat_heads__memory_aug_recurrent_mem_tr__sliding_local_dilated__prompt_kernel(
    A_x: jax.Array,
    A_mem0: jax.Array,
    A_Wq: jax.Array,
    A_Wk: jax.Array,
    A_Wv: jax.Array,
    A_Wo: jax.Array,
    A_seg_len: int,
    B_x: jax.Array,
    B_wqkv: jax.Array,
    B_wo: jax.Array,
):
    assert A_seg_len == SEG and A_x.shape == (1, S, D) and A_mem0.shape == (1, MEM, D)
    assert A_Wq.shape == (D, NH, 128) and A_Wo.shape == (NH, 128, D)
    assert B_x.shape == (1, S, D) and B_wqkv.shape == (D, 3 * D) and B_wo.shape == (D, D)

    hbm = pl.BlockSpec(memory_space=pl.ANY)
    out = pl.pallas_call(
        _kernel,
        out_shape=jax.ShapeDtypeStruct((S // SEG, SEG, 2 * D), bf16),
        in_specs=[hbm, pl.BlockSpec(memory_space=pltpu.VMEM)] + [hbm] * 7,
        out_specs=hbm,
        scratch_shapes=[
            _vmem((3 * NH, 512, 128)),
            _vmem((8, 2048, 128)),
            _vmem((8, S // 2, 128)),
            _vmem((NT_J, 64, D)),
            _vmem((3 * NG, 512, 128)),
            _vmem((8, 192, 128)),
            _vmem((8, 192, 128)),
            _vmem((ACT_TILES, 128, 128), f32),
            _vmem((ACT_TILES, 128, 128), f32),
            _vmem((NT_J, NG, 64, 128)),
            _vmem((8, 512, 128)),
            _vmem((NT_J, 64, D)),
            _vmem((NH, 8, 128)),
            _vmem((NH, 24, 128)),
            _vmem((NH, 24, 128)),
            _vmem((NH, 24, 128)),
            _vmem((8, 48, 128), f32),
            _vmem((8, 8, 128)),
            _vmem((S // SEG, SEG, D), bf16),
            pltpu.SMEM((1,), i32),
            pltpu.SemaphoreType.DMA((NT_J,)),
            pltpu.SemaphoreType.DMA((NG,)),
            pltpu.SemaphoreType.DMA((4,)),
            pltpu.SemaphoreType.DMA((2,)),
        ],
        compiler_params=pltpu.CompilerParams(vmem_limit_bytes=100 * 1024 * 1024),
    )(
        A_x.astype(bf16).reshape(S, D),
        A_mem0.astype(bf16).reshape(MEM, D),
        A_Wq.astype(bf16).reshape(D // 2, 2 * NH, 128),
        A_Wk.astype(bf16).reshape(D // 2, 2 * NH, 128),
        A_Wv.astype(bf16).reshape(D // 2, 2 * NH, 128),
        A_Wo.astype(bf16).reshape(NH * 128, D),
        B_x.astype(bf16).reshape(S // (2 * NT_J), 2 * NT_J, D),
        B_wqkv.astype(bf16),
        B_wo.astype(bf16),
    )
    return out.reshape(1, S, 2 * D)
```

```python
import functools

import jax
import jax.numpy as jnp
from jax import lax
import jax.experimental.pallas as pl
import jax.experimental.pallas.tpu as pltpu

f32 = jnp.float32
bf16 = jnp.bfloat16
i32 = jnp.int32

S = 2048
D = 1024
NH = 32
HG = 4
MEM = 8
SEG = 32
ROWS = MEM + SEG
UNROLL = 2
NSTEP = S // (UNROLL * SEG)
A_SCALE = 128 ** -0.5
LOG2E = 1.4426950408889634
B_SCALE = 32 ** -0.5 * LOG2E
WIN, DIL = 8, 2
NT_J = 16
NG = 8
HALO = WIN - 1
KV_TILES = HALO + NT_J
ACT_TILES = NT_J + 2 * KV_TILES + 1
MASKED = -1000000000.0
NEVER = -1e30

_NN = (((1,), (0,)), ((), ()))
_NT = (((1,), (1,)), ((), ()))


def _aligned(i, n):
    return i if isinstance(i, int) else pl.multiple_of(i, n)


def _as_bf16(x):
    return pltpu.bitcast(x, bf16)


def _as_i32(x):
    return pltpu.bitcast(x, i32)


def _interleave(a, b):
    def high(x):
        return pltpu.unpack_elementwise(x, index=1, packed_dtype=jnp.int16, unpacked_dtype=i32)

    def pack(x, y):
        return pltpu.pack_elementwise([x, y], packed_dtype=jnp.int16).astype(i32)

    return pack(a, b), pack(high(a), high(b))


def _mm(lhs, rhs, dims=_NN):
    return lax.dot_general(lhs, rhs, dims, preferred_element_type=f32)


def _a_keys(x):
    x = jnp.concatenate([x, jnp.zeros((-ROWS % 16, 128), f32)], axis=0).astype(bf16)
    return jnp.concatenate([x, jnp.zeros((128 - x.shape[0], 128), bf16)], axis=0)


def _a_probs(q, k):
    r = lax.broadcasted_iota(i32, (ROWS, 128), 0)
    c = lax.broadcasted_iota(i32, (ROWS, 128), 1)
    visible = (c < ROWS) & ((r < MEM) | (r >= c))
    s = jnp.where(visible, _mm(q, k, _NT) * A_SCALE, jnp.where(c < ROWS, MASKED, NEVER))
    e = jnp.exp(s - jnp.max(s, axis=1, keepdims=True))
    return e * (1.0 / jnp.sum(e, axis=1, keepdims=True))


def _kernel(ax_hbm, mem0_ref, wq_hbm, wk_hbm, wv_hbm, awo_hbm, bx_hbm, bw_hbm, bwo_hbm,
            out_hbm,
            W, WO, XA, XP, WB, WT0, WT1, ACT0, ACT1, OB, WOB, OUTB,
            H, OA, PART, OUTA, ZERO,
            sem_xp, sem_wb, sem_misc, sem_out):
    def slab_copy(src, col, dst, sem):
        return pltpu.make_async_copy(src.at[:, pl.ds(_aligned(col, 128), 128)],
                                     dst.bitcast(bf16), sem)

    def xp_copy(j):
        return pltpu.make_async_copy(bx_hbm.bitcast(i32).at[:, j, :], XP.at[j], sem_xp.at[j])

    def wb_copies(g):
        return [slab_copy(bw_hbm, t * D + g * 128, WB.at[3 * g + t], sem_wb.at[g])
                for t in range(3)]

    def w_copies(t):
        src = (wq_hbm, wk_hbm, wv_hbm)[t].bitcast(i32)
        return [pltpu.make_async_copy(src.at[:, 16 * e + i, :], W.at[3 * (2 * i + e) + t],
                                      sem_misc.at[3])
                for i in range(NH // 2) for e in range(2)]

    def wob_copies():
        return [slab_copy(bwo_hbm, c * 128, WOB.at[c], sem_misc.at[0]) for c in range(8)]

    def awo_copies():
        return [slab_copy(awo_hbm, c * 128, WO.at[c], sem_misc.at[1]) for c in range(8)]

    def xa_copies():
        return [slab_copy(ax_hbm, c * 128, XA.at[c], sem_misc.at[2]) for c in range(8)]

    def outb_copies():
        return [pltpu.make_async_copy(OUTB.at[j], out_hbm.bitcast(i32).at[:, j, pl.ds(D, D)],
                                      sem_out.at[0]) for j in range(NT_J)]

    def outa_copy(p):
        segs = pl.ds(UNROLL * p, UNROLL)
        return pltpu.make_async_copy(OUTA.at[segs], out_hbm.at[segs, :, pl.ds(0, D)],
                                     sem_out.at[1])

    def start(copies):
        for c in copies:
            c.start()

    def wait(copies):
        for c in copies:
            c.wait()

    def wait_all(buf, sem):
        pltpu.make_async_copy(buf, buf, sem).wait()

    def transpose_w(g, WT, items):
        for t, k in items:
            tile = _as_bf16(WB[3 * g + t, k * 64:(k + 1) * 64, :])
            WT[k, t * 64:(t + 1) * 64, :] = _as_i32(tile.T)

    def after(x, token):
        if token is None:
            return x
        token = pltpu.bitcast(jnp.concatenate([token] * (x.shape[0] // 8), axis=0), x.dtype)
        return jnp.where(jnp.full(x.shape, ZERO[0], i32) == 0, x, token)

    def act_tile(t, j):
        return j if t == 0 else NT_J + (t - 1) * KV_TILES + HALO + j

    def project(WT, ACT, j, t):
        lhs = _as_bf16(jnp.concatenate([WT[k, t * 64:(t + 1) * 64, :] for k in range(8)], axis=1))
        y = lax.dot_general(lhs, _as_bf16(XP[j]), _NT, preferred_element_type=f32)
        if t == 0:
            y = y * B_SCALE
        ACT[act_tile(t, j)] = y
        lane = lax.broadcasted_iota(i32, (128, 128), 1)
        if t == 2 and j == 0:
            ACT[ACT_TILES - 1] = jnp.where(lane == 0, y, pltpu.roll(y, 1, 1))
        if t > 0 and j >= NT_J - HALO:
            shifted = pltpu.roll(y, 2, 1)
            if t == 2:
                shifted = jnp.where(lane < 2, ACT[ACT_TILES - 1], shifted)
            ACT[act_tile(t, j - NT_J)] = shifted
        return y[0:8], y[120:128]

    def attend_head(ACT, j, hh, token):
        def load(t, jj):
            return ACT[act_tile(t, jj), hh * 32:(hh + 1) * 32, :]

        q = after(load(0, j), token)
        logits = []
        for w in range(WIN):
            lg = jnp.sum(q * load(1, j - w), axis=0, keepdims=True)
            if j < w:
                lg = jnp.where(lax.broadcasted_iota(i32, (1, 128), 1) < 2, MASKED * LOG2E, lg)
            logits.append(lg)
        m = functools.reduce(jnp.maximum, logits)
        es = [jnp.exp2(lg - m) for lg in logits]
        inv = 1.0 / functools.reduce(jnp.add, es)
        o = functools.reduce(jnp.add, [es[w] * load(2, j - w) for w in range(WIN)])
        return (o * inv).astype(bf16)

    def store_heads(g, j, heads):
        OB[j, g] = _as_i32(jnp.concatenate(heads, axis=0).T)

    def project_out(j, c):
        lhs = _as_bf16(jnp.concatenate([OB[j, g] for g in range(NG)], axis=1))
        y = jnp.dot(lhs, _as_bf16(WOB[c]), preferred_element_type=f32)
        OUTB[j, :, c * 128:(c + 1) * 128] = _as_i32(y.astype(bf16))
        return y[0:8], y[120:128]

    def split_heads(item, token):
        slab, part = divmod(item, 8)
        t, i = divmod(slab, NH // 2)
        rows = slice(part * 64, (part + 1) * 64)
        even, odd = 3 * (2 * i) + t, 3 * (2 * i + 1) + t
        W[even, rows, :], W[odd, rows, :] = _interleave(after(W[even, rows, :], token),
                                                        after(W[odd, rows, :], token))

    w_tiles = [(t, k) for t in range(3) for k in range(8)]

    def share(items, n, j):
        return items[len(items) * j // n:len(items) * (j + 1) // n]

    def xp_copies(lo, hi):
        return [xp_copy(j) for j in range(lo, hi)]

    start(wb_copies(0) + xp_copies(0, NT_J) + wb_copies(1) + wb_copies(2) + wb_copies(3))
    ZERO[0] = 0
    wait(wb_copies(0))
    transpose_w(0, WT0, w_tiles)

    def first_group_dma(j):
        if j in (0, 2, 6, 12):
            wait(xp_copies(j, {0: 2, 2: 6, 6: 12, 12: NT_J}[j]))
        if j == 12:
            wait(wb_copies(1))

    def group(g, parity, first=False, last=False, dma=None):
        wt, wt_next = (WT0, WT1)[parity], (WT0, WT1)[1 - parity]
        act, act_prev = (ACT0, ACT1)[parity], (ACT0, ACT1)[1 - parity]
        tokens = (None, None)
        for j in range(NT_J):
            if dma is not None:
                dma(j)
            heads = []
            for t in range(3):
                tokens, prev = project(wt, act, j, t), tokens
                if t == 0 and first and j >= 12:
                    transpose_w(1, wt_next, share(w_tiles, NT_J - 12, j - 12))
                if t == 0 and not first and not last:
                    transpose_w(g + 1, wt_next, share(w_tiles, NT_J, j))
                if not first:
                    heads += [attend_head(act_prev, j, hh, prev[when]) for hh, when in
                              (((0, 1),), ((1, 0),), ((2, 0), (3, 1)))[t]]
            if not first:
                store_heads(g - 1, j, heads)

    group(0, 0, first=True, dma=first_group_dma)

    def two_groups(i, carry):
        wait(wb_copies(2 * i + 2) + wb_copies(2 * i + 3))

        later = [c for g in range(4, NG) for c in wb_copies(g)] + wob_copies()
        for n, copies in enumerate((later + w_copies(0), w_copies(1) + awo_copies(),
                                    w_copies(2) + xa_copies())):
            pl.when(i == n)(functools.partial(start, copies))
        group(2 * i + 1, 1)
        group(2 * i + 2, 0)
        return carry

    lax.fori_loop(0, (NG - 2) // 2, two_groups, 0)
    group(NG - 1, 1, last=True)

    wait_all(WOB, sem_misc.at[0])
    wait_all(W, sem_misc.at[3])
    store_heads(NG - 1, 0, [attend_head(ACT1, 0, hh, None) for hh in range(4)])
    tokens = (None, None)
    w_items = list(range(3 * (NH // 2) * 8))
    for j in range(NT_J):
        heads = []
        for c in range(8):
            tokens, prev = project_out(j, c), tokens
            if j + 1 < NT_J and c % 2 == 0:
                heads.append(attend_head(ACT1, j + 1, c // 2, prev[0]))
            for item in share(w_items, NT_J * 8, j * 8 + c):
                split_heads(item, prev[1])
        if heads:
            store_heads(NG - 1, j + 1, heads)
    start(outb_copies())

    wait_all(WO, sem_misc.at[1])
    wait_all(XA, sem_misc.at[2])
    for c in range(8):
        H[c, 0:MEM, :] = mem0_ref[:, c * 128:(c + 1) * 128].astype(f32)

    def segment(s):
        rows = pl.ds(pl.multiple_of(s * (SEG // 2), SEG // 2), SEG // 2)
        for c in range(8):
            H[c, MEM:ROWS, :] = _as_bf16(XA[c, rows, :]).astype(f32)
        h_in = jnp.concatenate([H[c] for c in range(8)], axis=1)

        def proj(t, h):
            return _mm(h_in, _as_bf16(W[3 * h + t]))

        def out_part(h0, h1, c):
            o = jnp.concatenate([OA[h] for h in range(h0, h1)], axis=1)
            return _mm(o, _as_bf16(WO[c, h0 * 64:h1 * 64, :]))

        def finish(pending):
            for h, (prob, v) in pending.items():
                OA[h] = _mm(prob, v)

        pending = {}
        for g in range(NH // HG):
            heads = range(g * HG, (g + 1) * HG)
            q = {h: proj(0, h) for h in heads}
            k = {h: _a_keys(proj(1, h)) for h in heads}
            finish(pending)
            v = {h: _a_keys(proj(2, h)) for h in heads}
            pending = {h: (_a_probs(q[h], k[h]), v[h]) for h in heads}
        for c in range(4):
            PART[c] = out_part(0, NH // 2, c)
        finish(pending)
        for c in range(4, 8):
            PART[c] = out_part(0, NH // 2, c)
        for c in range(8):
            y = PART[c] + out_part(NH // 2, NH, c)
            H[c, 0:MEM, :] = y[0:MEM]
            OUTA[s, :, c * 128:(c + 1) * 128] = y[MEM:ROWS].astype(bf16)

    def step(p, carry):
        for u in range(UNROLL):
            segment(UNROLL * p + u)
        outa_copy(p).start()
        return carry

    lax.fori_loop(0, NSTEP, step, 0)

    wait_all(OUTB, sem_out.at[0])
    wait_all(OUTA, sem_out.at[1])


def _vmem(shape, dtype=i32):
    return pltpu.VMEM(shape, dtype)


@functools.partial(jax.jit, static_argnames=("A_seg_len",))
def pallas_concat_heads__memory_aug_recurrent_mem_tr__sliding_local_dilated__prompt_kernel(
    A_x: jax.Array,
    A_mem0: jax.Array,
    A_Wq: jax.Array,
    A_Wk: jax.Array,
    A_Wv: jax.Array,
    A_Wo: jax.Array,
    A_seg_len: int,
    B_x: jax.Array,
    B_wqkv: jax.Array,
    B_wo: jax.Array,
):
    assert A_seg_len == SEG and A_x.shape == (1, S, D) and A_mem0.shape == (1, MEM, D)
    assert A_Wq.shape == (D, NH, 128) and A_Wo.shape == (NH, 128, D)
    assert B_x.shape == (1, S, D) and B_wqkv.shape == (D, 3 * D) and B_wo.shape == (D, D)

    hbm = pl.BlockSpec(memory_space=pl.ANY)
    out = pl.pallas_call(
        _kernel,
        out_shape=jax.ShapeDtypeStruct((S // SEG, SEG, 2 * D), bf16),
        in_specs=[hbm, pl.BlockSpec(memory_space=pltpu.VMEM)] + [hbm] * 7,
        out_specs=hbm,
        scratch_shapes=[
            _vmem((3 * NH, 512, 128)),
            _vmem((8, 2048, 128)),
            _vmem((8, S // 2, 128)),
            _vmem((NT_J, 64, D)),
            _vmem((3 * NG, 512, 128)),
            _vmem((8, 192, 128)),
            _vmem((8, 192, 128)),
            _vmem((ACT_TILES, 128, 128), f32),
            _vmem((ACT_TILES, 128, 128), f32),
            _vmem((NT_J, NG, 64, 128)),
            _vmem((8, 512, 128)),
            _vmem((NT_J, 64, D)),
            _vmem((8, ROWS, 128), f32),
            _vmem((NH, ROWS, 128), f32),
            _vmem((8, ROWS, 128), f32),
            _vmem((S // SEG, SEG, D), bf16),
            pltpu.SMEM((1,), i32),
            pltpu.SemaphoreType.DMA((NT_J,)),
            pltpu.SemaphoreType.DMA((NG,)),
            pltpu.SemaphoreType.DMA((4,)),
            pltpu.SemaphoreType.DMA((2,)),
        ],
        compiler_params=pltpu.CompilerParams(vmem_limit_bytes=100 * 1024 * 1024),
    )(
        A_x.astype(bf16).reshape(S, D),
        A_mem0.astype(bf16).reshape(MEM, D),
        A_Wq.astype(bf16).reshape(D // 2, 2 * NH, 128),
        A_Wk.astype(bf16).reshape(D // 2, 2 * NH, 128),
        A_Wv.astype(bf16).reshape(D // 2, 2 * NH, 128),
        A_Wo.astype(bf16).reshape(NH * 128, D),
        B_x.astype(bf16).reshape(S // (2 * NT_J), 2 * NT_J, D),
        B_wqkv.astype(bf16),
        B_wo.astype(bf16),
    )
    return out.reshape(1, S, 2 * D)
```

```python
import functools

import jax
import jax.numpy as jnp
from jax import lax
import jax.experimental.pallas as pl
import jax.experimental.pallas.tpu as pltpu

f32 = jnp.float32
bf16 = jnp.bfloat16
i32 = jnp.int32

S = 2048
D = 1024
NH = 32
HG = 4
MEM = 8
SEG = 32
ROWS = MEM + SEG
UNROLL = 4
NSTEP = S // (UNROLL * SEG)
A_SCALE = 128 ** -0.5
LOG2E = 1.4426950408889634
B_SCALE = 32 ** -0.5 * LOG2E
WIN, DIL = 8, 2
NT_J = 16
NG = 8
HALO = WIN - 1
KV_TILES = HALO + NT_J
ACT_TILES = NT_J + 2 * KV_TILES + 1
MASKED = -1000000000.0
NEVER = -1e30

_NN = (((1,), (0,)), ((), ()))
_NT = (((1,), (1,)), ((), ()))


def _aligned(i, n):
    return i if isinstance(i, int) else pl.multiple_of(i, n)


def _as_bf16(x):
    return pltpu.bitcast(x, bf16)


def _as_i32(x):
    return pltpu.bitcast(x, i32)


def _interleave(a, b):
    def high(x):
        return pltpu.unpack_elementwise(x, index=1, packed_dtype=jnp.int16, unpacked_dtype=i32)

    def pack(x, y):
        return pltpu.pack_elementwise([x, y], packed_dtype=jnp.int16).astype(i32)

    return pack(a, b), pack(high(a), high(b))


def _mm(lhs, rhs, dims=_NN):
    return lax.dot_general(lhs, rhs, dims, preferred_element_type=f32)


def _a_keys(x):
    x = jnp.concatenate([x, jnp.zeros((-ROWS % 16, 128), f32)], axis=0).astype(bf16)
    return jnp.concatenate([x, jnp.zeros((128 - x.shape[0], 128), bf16)], axis=0)


def _a_probs(q, k):
    r = lax.broadcasted_iota(i32, (ROWS, 128), 0)
    c = lax.broadcasted_iota(i32, (ROWS, 128), 1)
    visible = (c < ROWS) & ((r < MEM) | (r >= c))
    s = jnp.where(visible, _mm(q, k, _NT) * A_SCALE, jnp.where(c < ROWS, MASKED, NEVER))
    e = jnp.exp(s - jnp.max(s, axis=1, keepdims=True))
    return e * (1.0 / jnp.sum(e, axis=1, keepdims=True))


def _kernel(ax_hbm, mem0_ref, wq_hbm, wk_hbm, wv_hbm, awo_hbm, bx_hbm, bw_hbm, bwo_hbm,
            out_hbm,
            W, WO, XA, XP, WB, WT0, WT1, ACT0, ACT1, OB, WOB, OUTB,
            H, OA, PART, HEAD, OUTA, ZERO,
            sem_xp, sem_wb, sem_misc, sem_out):
    def slab_copy(src, col, dst, sem):
        return pltpu.make_async_copy(src.at[:, pl.ds(_aligned(col, 128), 128)],
                                     dst.bitcast(bf16), sem)

    def xp_copy(j):
        return pltpu.make_async_copy(bx_hbm.bitcast(i32).at[:, j, :], XP.at[j], sem_xp.at[j])

    def wb_copies(g):
        return [slab_copy(bw_hbm, t * D + g * 128, WB.at[3 * g + t], sem_wb.at[g])
                for t in range(3)]

    def w_copies(t):
        src = (wq_hbm, wk_hbm, wv_hbm)[t].bitcast(i32)
        return [pltpu.make_async_copy(src.at[:, 16 * e + i, :], W.at[3 * (2 * i + e) + t],
                                      sem_misc.at[3])
                for i in range(NH // 2) for e in range(2)]

    def wob_copies():
        return [slab_copy(bwo_hbm, c * 128, WOB.at[c], sem_misc.at[0]) for c in range(8)]

    def awo_copies():
        return [slab_copy(awo_hbm, c * 128, WO.at[c], sem_misc.at[1]) for c in range(8)]

    def xa_copies():
        return [slab_copy(ax_hbm, c * 128, XA.at[c], sem_misc.at[2]) for c in range(8)]

    def outb_copies():
        return [pltpu.make_async_copy(OUTB.at[j], out_hbm.bitcast(i32).at[:, j, pl.ds(D, D)],
                                      sem_out.at[0]) for j in range(NT_J)]

    def outa_copy(p):
        segs = pl.ds(UNROLL * p, UNROLL)
        return pltpu.make_async_copy(OUTA.at[segs], out_hbm.at[segs, :, pl.ds(0, D)],
                                     sem_out.at[1])

    def start(copies):
        for c in copies:
            c.start()

    def wait(copies):
        for c in copies:
            c.wait()

    def wait_all(buf, sem):
        pltpu.make_async_copy(buf, buf, sem).wait()

    def transpose_w(g, WT, items):
        for t, k in items:
            tile = _as_bf16(WB[3 * g + t, k * 64:(k + 1) * 64, :])
            WT[k, t * 64:(t + 1) * 64, :] = _as_i32(tile.T)

    def after(x, token):
        if token is None:
            return x
        token = pltpu.bitcast(jnp.concatenate([token] * (x.shape[0] // 8), axis=0), x.dtype)
        return jnp.where(jnp.full(x.shape, ZERO[0], i32) == 0, x, token)

    def act_tile(t, j):
        return j if t == 0 else NT_J + (t - 1) * KV_TILES + HALO + j

    def project(WT, ACT, j, t):
        lhs = _as_bf16(jnp.concatenate([WT[k, t * 64:(t + 1) * 64, :] for k in range(8)], axis=1))
        y = lax.dot_general(lhs, _as_bf16(XP[j]), _NT, preferred_element_type=f32)
        if t == 0:
            y = y * B_SCALE
        ACT[act_tile(t, j)] = y
        lane = lax.broadcasted_iota(i32, (128, 128), 1)
        if t == 2 and j == 0:
            ACT[ACT_TILES - 1] = jnp.where(lane == 0, y, pltpu.roll(y, 1, 1))
        if t > 0 and j >= NT_J - HALO:
            shifted = pltpu.roll(y, 2, 1)
            if t == 2:
                shifted = jnp.where(lane < 2, ACT[ACT_TILES - 1], shifted)
            ACT[act_tile(t, j - NT_J)] = shifted
        return y[0:8], y[120:128]

    def attend_head(ACT, j, hh, token):
        def load(t, jj):
            return ACT[act_tile(t, jj), hh * 32:(hh + 1) * 32, :]

        q = after(load(0, j), token)
        logits = []
        for w in range(WIN):
            lg = jnp.sum(q * load(1, j - w), axis=0, keepdims=True)
            if j < w:
                lg = jnp.where(lax.broadcasted_iota(i32, (1, 128), 1) < 2, MASKED * LOG2E, lg)
            logits.append(lg)
        m = functools.reduce(jnp.maximum, logits)
        es = [jnp.exp2(lg - m) for lg in logits]
        inv = 1.0 / functools.reduce(jnp.add, es)
        o = functools.reduce(jnp.add, [es[w] * load(2, j - w) for w in range(WIN)])
        return (o * inv).astype(bf16)

    def store_heads(g, j, heads):
        OB[j, g] = _as_i32(jnp.concatenate(heads, axis=0).T)

    def project_out(j, c):
        lhs = _as_bf16(jnp.concatenate([OB[j, g] for g in range(NG)], axis=1))
        y = jnp.dot(lhs, _as_bf16(WOB[c]), preferred_element_type=f32)
        OUTB[j, :, c * 128:(c + 1) * 128] = _as_i32(y.astype(bf16))
        return y[0:8], y[120:128]

    def split_heads(item, token):
        slab, part = divmod(item, 8)
        t, i = divmod(slab, NH // 2)
        rows = slice(part * 64, (part + 1) * 64)
        even, odd = 3 * (2 * i) + t, 3 * (2 * i + 1) + t
        W[even, rows, :], W[odd, rows, :] = _interleave(after(W[even, rows, :], token),
                                                        W[odd, rows, :])

    w_tiles = [(t, k) for t in range(3) for k in range(8)]

    def share(items, n, j):
        return items[len(items) * j // n:len(items) * (j + 1) // n]

    def xp_copies(lo, hi):
        return [xp_copy(j) for j in range(lo, hi)]

    start(wb_copies(0) + xp_copies(0, NT_J) + wb_copies(1) + wb_copies(2) + wb_copies(3))
    ZERO[0] = 0
    wait(wb_copies(0))
    transpose_w(0, WT0, w_tiles)

    def first_group_dma(j):
        stages = (0, 2, 4, 7, 11, NT_J)
        if j in stages:
            wait(xp_copies(j, stages[stages.index(j) + 1]))
        if j == NT_J - 2:
            wait(wb_copies(1))

    def group(g, parity, first=False, last=False, dma=None):
        wt, wt_next = (WT0, WT1)[parity], (WT0, WT1)[1 - parity]
        act, act_prev = (ACT0, ACT1)[parity], (ACT0, ACT1)[1 - parity]
        tokens = (None, None)
        for j in range(NT_J):
            if dma is not None:
                dma(j)
            heads = []
            for t in range(3):
                tokens, prev = project(wt, act, j, t), tokens
                if first and j >= NT_J - 2:
                    transpose_w(1, wt_next, share(w_tiles, 6, 3 * (j - NT_J + 2) + t))
                if t == 0 and not first and not last:
                    transpose_w(g + 1, wt_next, share(w_tiles, NT_J, j))
                if not first:
                    heads += [attend_head(act_prev, j, hh, prev[when]) for hh, when in
                              (((0, 1),), ((1, 0),), ((2, 0), (3, 1)))[t]]
            if not first:
                store_heads(g - 1, j, heads)

    group(0, 0, first=True, dma=first_group_dma)

    def two_groups(i, carry):
        wait(wb_copies(2 * i + 2) + wb_copies(2 * i + 3))

        later = [c for g in range(4, NG) for c in wb_copies(g)] + wob_copies()
        for n, copies in enumerate((later + w_copies(0), w_copies(1) + awo_copies(),
                                    w_copies(2) + xa_copies())):
            pl.when(i == n)(functools.partial(start, copies))
        group(2 * i + 1, 1)
        group(2 * i + 2, 0)
        return carry

    lax.fori_loop(0, (NG - 2) // 2, two_groups, 0)
    group(NG - 1, 1, last=True)

    wait_all(WOB, sem_misc.at[0])
    wait_all(W, sem_misc.at[3])
    store_heads(NG - 1, 0, [attend_head(ACT1, 0, hh, None) for hh in range(4)])
    tokens = (None, None)
    w_items = list(range(3 * (NH // 2) * 8))
    for j in range(NT_J):
        heads = []
        for c in range(8):
            tokens, prev = project_out(j, c), tokens
            if j + 1 < NT_J and c % 2 == 0:
                heads.append(attend_head(ACT1, j + 1, c // 2, prev[0]))
            for item in share(w_items, NT_J * 8 - 4, j * 8 + c):
                split_heads(item, prev[item % 2])
        if heads:
            store_heads(NG - 1, j + 1, heads)
    start(outb_copies())

    wait_all(WO, sem_misc.at[1])
    wait_all(XA, sem_misc.at[2])
    for c in range(8):
        H[c, 0:MEM, :] = mem0_ref[:, c * 128:(c + 1) * 128].astype(f32)

    def segment(s):
        rows = pl.ds(pl.multiple_of(s * (SEG // 2), SEG // 2), SEG // 2)
        for c in range(8):
            H[c, MEM:ROWS, :] = _as_bf16(XA[c, rows, :]).astype(f32)
        h_in = jnp.concatenate([H[c] for c in range(8)], axis=1)

        def proj(t, h):
            return _mm(h_in, _as_bf16(W[3 * h + t]))

        def out_part(h0, h1, c):
            o = jnp.concatenate([OA[h] for h in range(h0, h1)], axis=1)
            return _mm(o, _as_bf16(WO[c, h0 * 64:h1 * 64, :]))

        def finish(pending):
            for h, (prob, v) in pending.items():
                OA[h] = _mm(prob, v)

        pending = {}
        for g in range(NH // HG):
            heads = range(g * HG, (g + 1) * HG)
            if g == 0:
                for h in heads:
                    HEAD[h] = _mm(h_in[:, :D // 2], _as_bf16(W[3 * h, 0:256, :]))
                q = {h: HEAD[h] + _mm(h_in[:, D // 2:], _as_bf16(W[3 * h, 256:512, :]))
                     for h in heads}
            else:
                q = {h: proj(0, h) for h in heads}
            k = {h: _a_keys(proj(1, h)) for h in heads}
            finish(pending)
            v = {h: _a_keys(proj(2, h)) for h in heads}
            pending = {h: (_a_probs(q[h], k[h]), v[h]) for h in heads}
        for c in range(4):
            PART[c] = out_part(0, NH // 2, c)
        finish(pending)
        for c in range(4, 8):
            PART[c] = out_part(0, NH // 2, c)
        for c in range(8):
            y = PART[c] + out_part(NH // 2, NH, c)
            H[c, 0:MEM, :] = y[0:MEM]
            OUTA[s, :, c * 128:(c + 1) * 128] = y[MEM:ROWS].astype(bf16)

    def step(p, carry):
        for u in range(UNROLL):
            segment(UNROLL * p + u)
        outa_copy(p).start()
        return carry

    lax.fori_loop(0, NSTEP, step, 0)

    wait_all(OUTB, sem_out.at[0])
    wait_all(OUTA, sem_out.at[1])


def _vmem(shape, dtype=i32):
    return pltpu.VMEM(shape, dtype)


@functools.partial(jax.jit, static_argnames=("A_seg_len",))
def pallas_concat_heads__memory_aug_recurrent_mem_tr__sliding_local_dilated__prompt_kernel(
    A_x: jax.Array,
    A_mem0: jax.Array,
    A_Wq: jax.Array,
    A_Wk: jax.Array,
    A_Wv: jax.Array,
    A_Wo: jax.Array,
    A_seg_len: int,
    B_x: jax.Array,
    B_wqkv: jax.Array,
    B_wo: jax.Array,
):
    assert A_seg_len == SEG and A_x.shape == (1, S, D) and A_mem0.shape == (1, MEM, D)
    assert A_Wq.shape == (D, NH, 128) and A_Wo.shape == (NH, 128, D)
    assert B_x.shape == (1, S, D) and B_wqkv.shape == (D, 3 * D) and B_wo.shape == (D, D)

    hbm = pl.BlockSpec(memory_space=pl.ANY)
    out = pl.pallas_call(
        _kernel,
        out_shape=jax.ShapeDtypeStruct((S // SEG, SEG, 2 * D), bf16),
        in_specs=[hbm, pl.BlockSpec(memory_space=pltpu.VMEM)] + [hbm] * 7,
        out_specs=hbm,
        scratch_shapes=[
            _vmem((3 * NH, 512, 128)),
            _vmem((8, 2048, 128)),
            _vmem((8, S // 2, 128)),
            _vmem((NT_J, 64, D)),
            _vmem((3 * NG, 512, 128)),
            _vmem((8, 192, 128)),
            _vmem((8, 192, 128)),
            _vmem((ACT_TILES, 128, 128), f32),
            _vmem((ACT_TILES, 128, 128), f32),
            _vmem((NT_J, NG, 64, 128)),
            _vmem((8, 512, 128)),
            _vmem((NT_J, 64, D)),
            _vmem((8, ROWS, 128), f32),
            _vmem((NH, ROWS, 128), f32),
            _vmem((8, ROWS, 128), f32),
            _vmem((HG, ROWS, 128), f32),
            _vmem((S // SEG, SEG, D), bf16),
            pltpu.SMEM((1,), i32),
            pltpu.SemaphoreType.DMA((NT_J,)),
            pltpu.SemaphoreType.DMA((NG,)),
            pltpu.SemaphoreType.DMA((4,)),
            pltpu.SemaphoreType.DMA((2,)),
        ],
        compiler_params=pltpu.CompilerParams(vmem_limit_bytes=100 * 1024 * 1024),
    )(
        A_x.astype(bf16).reshape(S, D),
        A_mem0.astype(bf16).reshape(MEM, D),
        A_Wq.astype(bf16).reshape(D // 2, 2 * NH, 128),
        A_Wk.astype(bf16).reshape(D // 2, 2 * NH, 128),
        A_Wv.astype(bf16).reshape(D // 2, 2 * NH, 128),
        A_Wo.astype(bf16).reshape(NH * 128, D),
        B_x.astype(bf16).reshape(S // (2 * NT_J), 2 * NT_J, D),
        B_wqkv.astype(bf16),
        B_wo.astype(bf16),
    )
    return out.reshape(1, S, 2 * D)
```

```python
import functools

import jax
import jax.numpy as jnp
from jax import lax
import jax.experimental.pallas as pl
import jax.experimental.pallas.tpu as pltpu

f32 = jnp.float32
bf16 = jnp.bfloat16
i32 = jnp.int32

S = 2048
D = 1024
NH = 32
HG = 4
MEM = 8
SEG = 32
ROWS = MEM + SEG
UNROLL = 4
NSTEP = S // (UNROLL * SEG)
A_SCALE = 128 ** -0.5
LOG2E = 1.4426950408889634
B_SCALE = 32 ** -0.5 * LOG2E
WIN = 8
NT_J = 16
NG = 8
HALO = WIN - 1
KV_TILES = HALO + NT_J
ACT_TILES = NT_J + 2 * KV_TILES + 1
MASKED = -1000000000.0
NEVER = -1e30

_NN = (((1,), (0,)), ((), ()))
_NT = (((1,), (1,)), ((), ()))


def _aligned(i, n):
    return i if isinstance(i, int) else pl.multiple_of(i, n)


def _as_bf16(x):
    return pltpu.bitcast(x, bf16)


def _as_i32(x):
    return pltpu.bitcast(x, i32)


def _interleave(a, b):
    def high(x):
        return pltpu.unpack_elementwise(x, index=1, packed_dtype=jnp.int16, unpacked_dtype=i32)

    def pack(x, y):
        return pltpu.pack_elementwise([x, y], packed_dtype=jnp.int16).astype(i32)

    return pack(a, b), pack(high(a), high(b))


def _mm(lhs, rhs, dims=_NN):
    return lax.dot_general(lhs, rhs, dims, preferred_element_type=f32)


def _a_keys(x):
    x = jnp.concatenate([x, jnp.zeros((-ROWS % 16, 128), f32)], axis=0).astype(bf16)
    return jnp.concatenate([x, jnp.zeros((128 - x.shape[0], 128), bf16)], axis=0)


def _a_probs(q, k):
    r = lax.broadcasted_iota(i32, (ROWS, 128), 0)
    c = lax.broadcasted_iota(i32, (ROWS, 128), 1)
    visible = (c < ROWS) & ((r < MEM) | (r >= c))
    s = jnp.where(visible, _mm(q, k, _NT) * A_SCALE, jnp.where(c < ROWS, MASKED, NEVER))
    e = jnp.exp(s - jnp.max(s, axis=1, keepdims=True))
    return e * (1.0 / jnp.sum(e, axis=1, keepdims=True))


def _kernel(ax_hbm, mem0_hbm, wq_hbm, wk_hbm, wv_hbm, awo_hbm, bx_hbm, bw_hbm, bwo_hbm,
            out_hbm,
            W, WO, XA, XP, WB, WT0, WT1, ACT0, ACT1, OB, WOB, OUTB,
            MEM0, H, OA, PART, HEAD, OUTA, ZERO,
            sem_xp, sem_wb, sem_misc, sem_out):
    def slab_copy(src, col, dst, sem):
        return pltpu.make_async_copy(src.at[:, pl.ds(_aligned(col, 128), 128)],
                                     dst.bitcast(bf16), sem)

    def xp_copy(j):
        return pltpu.make_async_copy(bx_hbm.bitcast(i32).at[:, j, :], XP.at[j], sem_xp.at[j])

    def wb_copies(g):
        return [slab_copy(bw_hbm, t * D + g * 128, WB.at[3 * g + t], sem_wb.at[g])
                for t in range(3)]

    def w_copies(t):
        src = (wq_hbm, wk_hbm, wv_hbm)[t].bitcast(i32)
        return [pltpu.make_async_copy(src.at[:, 16 * e + i, :], W.at[3 * (2 * i + e) + t],
                                      sem_misc.at[3])
                for i in range(NH // 2) for e in range(2)]

    def wob_copies():
        return [slab_copy(bwo_hbm, c * 128, WOB.at[c], sem_misc.at[0]) for c in range(8)]

    def awo_copies():
        return [slab_copy(awo_hbm, c * 128, WO.at[c], sem_misc.at[1]) for c in range(8)]

    def xa_copies():
        return [slab_copy(ax_hbm, c * 128, XA.at[c], sem_misc.at[2]) for c in range(8)]

    def mem0_copy():
        return pltpu.make_async_copy(mem0_hbm, MEM0, sem_misc.at[4])

    def outb_copies():
        return [pltpu.make_async_copy(OUTB.at[j], out_hbm.bitcast(i32).at[:, j, pl.ds(D, D)],
                                      sem_out.at[0]) for j in range(NT_J)]

    def outa_copy(p):
        segs = pl.ds(UNROLL * p, UNROLL)
        return pltpu.make_async_copy(OUTA.at[segs], out_hbm.at[segs, :, pl.ds(0, D)],
                                     sem_out.at[1])

    def start(copies):
        for c in copies:
            c.start()

    def wait(copies):
        for c in copies:
            c.wait()

    def wait_all(buf, sem):
        pltpu.make_async_copy(buf, buf, sem).wait()

    def transpose_w(g, WT, items):
        for t, k in items:
            tile = _as_bf16(WB[3 * g + t, k * 64:(k + 1) * 64, :])
            WT[k, t * 64:(t + 1) * 64, :] = _as_i32(tile.T)

    def after(x, token):
        if token is None:
            return x
        token = pltpu.bitcast(jnp.concatenate([token] * (x.shape[0] // 8), axis=0), x.dtype)
        return jnp.where(jnp.full(x.shape, ZERO[0], i32) == 0, x, token)

    def act_tile(t, j):
        return j if t == 0 else NT_J + (t - 1) * KV_TILES + HALO + j

    def project(WT, ACT, j, t):
        lhs = _as_bf16(jnp.concatenate([WT[k, t * 64:(t + 1) * 64, :] for k in range(8)], axis=1))
        y = lax.dot_general(lhs, _as_bf16(XP[j]), _NT, preferred_element_type=f32)
        if t == 0:
            y = y * B_SCALE
        ACT[act_tile(t, j)] = y
        lane = lax.broadcasted_iota(i32, (128, 128), 1)
        if t == 2 and j == 0:
            ACT[ACT_TILES - 1] = jnp.where(lane == 0, y, pltpu.roll(y, 1, 1))
        if t > 0 and j >= NT_J - HALO:
            shifted = pltpu.roll(y, 2, 1)
            if t == 2:
                shifted = jnp.where(lane < 2, ACT[ACT_TILES - 1], shifted)
            ACT[act_tile(t, j - NT_J)] = shifted
        return y[0:8], y[120:128]

    def attend_head(ACT, j, hh, token):
        def load(t, jj):
            return ACT[act_tile(t, jj), hh * 32:(hh + 1) * 32, :]

        q = after(load(0, j), token)
        logits = []
        for w in range(WIN):
            lg = jnp.sum(q * load(1, j - w), axis=0, keepdims=True)
            if j < w:
                lg = jnp.where(lax.broadcasted_iota(i32, (1, 128), 1) < 2, MASKED * LOG2E, lg)
            logits.append(lg)
        m = functools.reduce(jnp.maximum, logits)
        es = [jnp.exp2(lg - m) for lg in logits]
        inv = 1.0 / functools.reduce(jnp.add, es)
        o = functools.reduce(jnp.add, [es[w] * load(2, j - w) for w in range(WIN)])
        return (o * inv).astype(bf16)

    def store_heads(g, j, heads):
        OB[j, g] = _as_i32(jnp.concatenate(heads, axis=0).T)

    def project_out(j, c):
        lhs = _as_bf16(jnp.concatenate([OB[j, g] for g in range(NG)], axis=1))
        y = jnp.dot(lhs, _as_bf16(WOB[c]), preferred_element_type=f32)
        OUTB[j, :, c * 128:(c + 1) * 128] = _as_i32(y.astype(bf16))
        return y[0:8], y[120:128]

    def split_heads(item, token):
        slab, part = divmod(item, 8)
        t, i = divmod(slab, NH // 2)
        rows = slice(part * 64, (part + 1) * 64)
        even, odd = 3 * (2 * i) + t, 3 * (2 * i + 1) + t
        W[even, rows, :], W[odd, rows, :] = _interleave(after(W[even, rows, :], token),
                                                        W[odd, rows, :])

    w_tiles = [(t, k) for t in range(3) for k in range(8)]

    def share(items, n, j):
        return items[len(items) * j // n:len(items) * (j + 1) // n]

    def xp_copies(lo, hi):
        return [xp_copy(j) for j in range(lo, hi)]

    start(wb_copies(0) + xp_copies(0, NT_J) + wb_copies(1) + wb_copies(2) + wb_copies(3))
    ZERO[0] = 0
    wait(wb_copies(0))
    transpose_w(0, WT0, w_tiles)

    def first_group_dma(j):
        stages = (0, 2, 4, 7, 11, NT_J)
        if j in stages:
            wait(xp_copies(j, stages[stages.index(j) + 1]))
        if j == NT_J - 2:
            wait(wb_copies(1))

    def group(g, parity, first=False, last=False, dma=None):
        wt, wt_next = (WT0, WT1)[parity], (WT0, WT1)[1 - parity]
        act, act_prev = (ACT0, ACT1)[parity], (ACT0, ACT1)[1 - parity]
        tokens = (None, None)
        for j in range(NT_J):
            if dma is not None:
                dma(j)
            heads = []
            for t in range(3):
                tokens, prev = project(wt, act, j, t), tokens
                if first and j >= NT_J - 2:
                    transpose_w(1, wt_next, share(w_tiles, 6, 3 * (j - NT_J + 2) + t))
                if t == 0 and not first and not last:
                    transpose_w(g + 1, wt_next, share(w_tiles, NT_J, j))
                if not first:
                    heads += [attend_head(act_prev, j, hh, prev[when]) for hh, when in
                              (((0, 1),), ((1, 0),), ((2, 0), (3, 1)))[t]]
            if not first:
                store_heads(g - 1, j, heads)

    group(0, 0, first=True, dma=first_group_dma)

    def two_groups(i, carry):
        wait(wb_copies(2 * i + 2) + wb_copies(2 * i + 3))

        later = [c for g in range(4, NG) for c in wb_copies(g)] + wob_copies()
        for n, copies in enumerate((later + w_copies(0), w_copies(1) + awo_copies(),
                                    w_copies(2) + xa_copies() + [mem0_copy()])):
            pl.when(i == n)(functools.partial(start, copies))
        group(2 * i + 1, 1)
        group(2 * i + 2, 0)
        return carry

    lax.fori_loop(0, (NG - 2) // 2, two_groups, 0)
    group(NG - 1, 1, last=True)

    wait_all(WOB, sem_misc.at[0])
    wait_all(W, sem_misc.at[3])
    store_heads(NG - 1, 0, [attend_head(ACT1, 0, hh, None) for hh in range(4)])
    tokens = (None, None)
    w_items = list(range(3 * (NH // 2) * 8))
    for j in range(NT_J):
        heads = []
        for c in range(8):
            tokens, prev = project_out(j, c), tokens
            if j + 1 < NT_J and c % 2 == 0:
                heads.append(attend_head(ACT1, j + 1, c // 2, prev[0]))
            for item in share(w_items, NT_J * 8 - 4, j * 8 + c):
                split_heads(item, prev[item % 2])
        if heads:
            store_heads(NG - 1, j + 1, heads)
    start(outb_copies())

    wait_all(WO, sem_misc.at[1])
    wait_all(XA, sem_misc.at[2])
    mem0_copy().wait()
    for c in range(8):
        H[c, 0:MEM, :] = MEM0[:, c * 128:(c + 1) * 128].astype(f32)

    def segment(s):
        rows = pl.ds(pl.multiple_of(s * (SEG // 2), SEG // 2), SEG // 2)
        for c in range(8):
            H[c, MEM:ROWS, :] = _as_bf16(XA[c, rows, :]).astype(f32)
        h_in = jnp.concatenate([H[c] for c in range(8)], axis=1)

        def proj(t, h):
            return _mm(h_in, _as_bf16(W[3 * h + t]))

        def out_part(h0, h1, c):
            o = jnp.concatenate([OA[h] for h in range(h0, h1)], axis=1)
            return _mm(o, _as_bf16(WO[c, h0 * 64:h1 * 64, :]))

        def finish(pending):
            for h, (prob, v) in pending.items():
                OA[h] = _mm(prob, v)

        pending = {}
        for g in range(NH // HG):
            heads = range(g * HG, (g + 1) * HG)
            if g == 0:
                for h in heads:
                    HEAD[h] = _mm(h_in[:, :D // 2], _as_bf16(W[3 * h, 0:256, :]))
                q = {h: HEAD[h] + _mm(h_in[:, D // 2:], _as_bf16(W[3 * h, 256:512, :]))
                     for h in heads}
            else:
                q = {h: proj(0, h) for h in heads}
            k = {h: _a_keys(proj(1, h)) for h in heads}
            finish(pending)
            v = {h: _a_keys(proj(2, h)) for h in heads}
            pending = {h: (_a_probs(q[h], k[h]), v[h]) for h in heads}
        for c in range(4):
            PART[c] = out_part(0, NH // 2, c)
        finish(pending)
        for c in range(4, 8):
            PART[c] = out_part(0, NH // 2, c)
        for c in range(8):
            y = PART[c] + out_part(NH // 2, NH, c)
            H[c, 0:MEM, :] = y[0:MEM]
            OUTA[s, :, c * 128:(c + 1) * 128] = y[MEM:ROWS].astype(bf16)

    def step(p, carry):
        for u in range(UNROLL):
            segment(UNROLL * p + u)
        outa_copy(p).start()
        return carry

    lax.fori_loop(0, NSTEP, step, 0)

    wait_all(OUTB, sem_out.at[0])
    wait_all(OUTA, sem_out.at[1])


def _vmem(shape, dtype=i32):
    return pltpu.VMEM(shape, dtype)


@functools.partial(jax.jit, static_argnames=("A_seg_len",))
def pallas_concat_heads__memory_aug_recurrent_mem_tr__sliding_local_dilated__prompt_kernel(
    A_x: jax.Array,
    A_mem0: jax.Array,
    A_Wq: jax.Array,
    A_Wk: jax.Array,
    A_Wv: jax.Array,
    A_Wo: jax.Array,
    A_seg_len: int,
    B_x: jax.Array,
    B_wqkv: jax.Array,
    B_wo: jax.Array,
):
    assert A_seg_len == SEG and A_x.shape == (1, S, D) and A_mem0.shape == (1, MEM, D)
    assert A_Wq.shape == (D, NH, 128) and A_Wo.shape == (NH, 128, D)
    assert B_x.shape == (1, S, D) and B_wqkv.shape == (D, 3 * D) and B_wo.shape == (D, D)

    hbm = pl.BlockSpec(memory_space=pl.ANY)
    out = pl.pallas_call(
        _kernel,
        out_shape=jax.ShapeDtypeStruct((S // SEG, SEG, 2 * D), bf16),
        in_specs=[hbm] * 9,
        out_specs=hbm,
        scratch_shapes=[
            _vmem((3 * NH, 512, 128)),
            _vmem((8, 2048, 128)),
            _vmem((8, S // 2, 128)),
            _vmem((NT_J, 64, D)),
            _vmem((3 * NG, 512, 128)),
            _vmem((8, 192, 128)),
            _vmem((8, 192, 128)),
            _vmem((ACT_TILES, 128, 128), f32),
            _vmem((ACT_TILES, 128, 128), f32),
            _vmem((NT_J, NG, 64, 128)),
            _vmem((8, 512, 128)),
            _vmem((NT_J, 64, D)),
            _vmem((MEM, D), bf16),
            _vmem((8, ROWS, 128), f32),
            _vmem((NH, ROWS, 128), f32),
            _vmem((8, ROWS, 128), f32),
            _vmem((HG, ROWS, 128), f32),
            _vmem((S // SEG, SEG, D), bf16),
            pltpu.SMEM((1,), i32),
            pltpu.SemaphoreType.DMA((NT_J,)),
            pltpu.SemaphoreType.DMA((NG,)),
            pltpu.SemaphoreType.DMA((5,)),
            pltpu.SemaphoreType.DMA((2,)),
        ],
        compiler_params=pltpu.CompilerParams(vmem_limit_bytes=100 * 1024 * 1024),
    )(
        A_x.astype(bf16).reshape(S, D),
        A_mem0.astype(bf16).reshape(MEM, D),
        A_Wq.astype(bf16).reshape(D // 2, 2 * NH, 128),
        A_Wk.astype(bf16).reshape(D // 2, 2 * NH, 128),
        A_Wv.astype(bf16).reshape(D // 2, 2 * NH, 128),
        A_Wo.astype(bf16).reshape(NH * 128, D),
        B_x.astype(bf16).reshape(S // (2 * NT_J), 2 * NT_J, D),
        B_wqkv.astype(bf16),
        B_wo.astype(bf16),
    )
    return out.reshape(1, S, 2 * D)
```

```python
import functools

import jax
import jax.numpy as jnp
from jax import lax
import jax.experimental.pallas as pl
import jax.experimental.pallas.tpu as pltpu

f32 = jnp.float32
bf16 = jnp.bfloat16
i32 = jnp.int32

S = 2048
D = 1024
NH = 32
HG = 4
MEM = 8
SEG = 32
ROWS = MEM + SEG
UNROLL = 4
NSTEP = S // (UNROLL * SEG)
A_SCALE = 128 ** -0.5
LOG2E = 1.4426950408889634
B_SCALE = 32 ** -0.5 * LOG2E
WIN = 8
NT_J = 16
NG = 8
HALO = WIN - 1
KV_TILES = HALO + NT_J
ACT_TILES = NT_J + 2 * KV_TILES + 1
MASKED = -1000000000.0
NEVER = -1e30

_NN = (((1,), (0,)), ((), ()))
_NT = (((1,), (1,)), ((), ()))


def _aligned(i, n):
    return i if isinstance(i, int) else pl.multiple_of(i, n)


def _as_bf16(x):
    return pltpu.bitcast(x, bf16)


def _as_i32(x):
    return pltpu.bitcast(x, i32)


def _interleave(a, b):
    return (a & 0xFFFF) | (b << 16), lax.shift_right_logical(a, 16) | (b & -65536)


def _mm(lhs, rhs, dims=_NN):
    return lax.dot_general(lhs, rhs, dims, preferred_element_type=f32)


def _a_keys(x):
    x = jnp.concatenate([x, jnp.zeros((-ROWS % 16, 128), f32)], axis=0).astype(bf16)
    return jnp.concatenate([x, jnp.zeros((128 - x.shape[0], 128), bf16)], axis=0)


def _a_probs(q, k):
    r = lax.broadcasted_iota(i32, (ROWS, 128), 0)
    c = lax.broadcasted_iota(i32, (ROWS, 128), 1)
    visible = (c < ROWS) & ((r < MEM) | (r >= c))
    s = jnp.where(visible, _mm(q, k, _NT) * A_SCALE, jnp.where(c < ROWS, MASKED, NEVER))
    e = jnp.exp(s - jnp.max(s, axis=1, keepdims=True))
    return e * (1.0 / jnp.sum(e, axis=1, keepdims=True))


def _kernel(ax_hbm, mem0_hbm, wq_hbm, wk_hbm, wv_hbm, awo_hbm, bx_hbm, bw_hbm, bwo_hbm,
            out_hbm,
            W, WO, XA, XP, WB, WT0, WT1, ACT0, ACT1, OB, WOB, OUTB,
            MEM0, H, OA, PART, HEAD, OUTA, ZERO,
            sem_xp, sem_wb, sem_misc, sem_out):
    def slab_copy(src, col, dst, sem):
        return pltpu.make_async_copy(src.at[:, pl.ds(_aligned(col, 128), 128)],
                                     dst.bitcast(bf16), sem)

    def xp_copy(j):
        return pltpu.make_async_copy(bx_hbm.bitcast(i32).at[:, j, :], XP.at[j], sem_xp.at[j])

    def wb_copies(g):
        return [slab_copy(bw_hbm, t * D + g * 128, WB.at[3 * g + t], sem_wb.at[g])
                for t in range(3)]

    def w_copies(t):
        src = (wq_hbm, wk_hbm, wv_hbm)[t].bitcast(i32)
        return [pltpu.make_async_copy(src.at[:, 16 * e + i, :], W.at[3 * (2 * i + e) + t],
                                      sem_misc.at[3])
                for i in range(NH // 2) for e in range(2)]

    def wob_copies():
        return [slab_copy(bwo_hbm, c * 128, WOB.at[c], sem_misc.at[0]) for c in range(8)]

    def awo_copies():
        return [slab_copy(awo_hbm, c * 128, WO.at[c], sem_misc.at[1]) for c in range(8)]

    def xa_copies():
        return [slab_copy(ax_hbm, c * 128, XA.at[c], sem_misc.at[2]) for c in range(8)]

    def mem0_copy():
        return pltpu.make_async_copy(mem0_hbm, MEM0, sem_misc.at[4])

    def outb_copies():
        return [pltpu.make_async_copy(OUTB.at[j], out_hbm.bitcast(i32).at[:, j, pl.ds(D, D)],
                                      sem_out.at[0]) for j in range(NT_J)]

    def outa_copy(p):
        segs = pl.ds(UNROLL * p, UNROLL)
        return pltpu.make_async_copy(OUTA.at[segs], out_hbm.at[segs, :, pl.ds(0, D)],
                                     sem_out.at[1])

    def start(copies):
        for c in copies:
            c.start()

    def wait(copies):
        for c in copies:
            c.wait()

    def wait_all(buf, sem):
        pltpu.make_async_copy(buf, buf, sem).wait()

    def transpose_w(g, WT, items):
        for t, k in items:
            tile = _as_bf16(WB[3 * g + t, k * 64:(k + 1) * 64, :])
            WT[k, t * 64:(t + 1) * 64, :] = _as_i32(tile.T)

    def after(x, token):
        if token is None:
            return x
        token = pltpu.bitcast(jnp.concatenate([token] * (x.shape[0] // 8), axis=0), x.dtype)
        return jnp.where(jnp.full(x.shape, ZERO[0], i32) == 0, x, token)

    def act_tile(t, j):
        return j if t == 0 else NT_J + (t - 1) * KV_TILES + HALO + j

    def project(WT, ACT, j, t):
        lhs = _as_bf16(jnp.concatenate([WT[k, t * 64:(t + 1) * 64, :] for k in range(8)], axis=1))
        y = lax.dot_general(lhs, _as_bf16(XP[j]), _NT, preferred_element_type=f32)
        if t == 0:
            y = y * B_SCALE
        ACT[act_tile(t, j)] = y
        lane = lax.broadcasted_iota(i32, (128, 128), 1)
        if t == 2 and j == 0:
            ACT[ACT_TILES - 1] = jnp.where(lane == 0, y, pltpu.roll(y, 1, 1))
        if t > 0 and j >= NT_J - HALO:
            shifted = pltpu.roll(y, 2, 1)
            if t == 2:
                shifted = jnp.where(lane < 2, ACT[ACT_TILES - 1], shifted)
            ACT[act_tile(t, j - NT_J)] = shifted
        return y[0:8], y[120:128]

    def attend_head(ACT, j, hh, token):
        def load(t, jj):
            return ACT[act_tile(t, jj), hh * 32:(hh + 1) * 32, :]

        q = after(load(0, j), token)
        logits = []
        for w in range(WIN):
            lg = jnp.sum(q * load(1, j - w), axis=0, keepdims=True)
            if j < w:
                lg = jnp.where(lax.broadcasted_iota(i32, (1, 128), 1) < 2, MASKED * LOG2E, lg)
            logits.append(lg)
        m = functools.reduce(jnp.maximum, logits)
        es = [jnp.exp2(lg - m) for lg in logits]
        inv = 1.0 / functools.reduce(jnp.add, es)
        o = functools.reduce(jnp.add, [es[w] * load(2, j - w) for w in range(WIN)])
        return (o * inv).astype(bf16)

    def store_heads(g, j, heads):
        OB[j, g] = _as_i32(jnp.concatenate(heads, axis=0).T)

    def project_out(j, c):
        lhs = _as_bf16(jnp.concatenate([OB[j, g] for g in range(NG)], axis=1))
        y = jnp.dot(lhs, _as_bf16(WOB[c]), preferred_element_type=f32)
        OUTB[j, :, c * 128:(c + 1) * 128] = _as_i32(y.astype(bf16))
        return y[0:8], y[120:128]

    def split_heads(item, token):
        slab, part = divmod(item, 8)
        t, i = divmod(slab, NH // 2)
        rows = slice(part * 64, (part + 1) * 64)
        even, odd = 3 * (2 * i) + t, 3 * (2 * i + 1) + t
        W[even, rows, :], W[odd, rows, :] = _interleave(after(W[even, rows, :], token),
                                                        W[odd, rows, :])

    w_tiles = [(t, k) for t in range(3) for k in range(8)]

    def share(items, n, j):
        return items[len(items) * j // n:len(items) * (j + 1) // n]

    def xp_copies(lo, hi):
        return [xp_copy(j) for j in range(lo, hi)]

    start(wb_copies(0) + xp_copies(0, NT_J) + wb_copies(1) + wb_copies(2) + wb_copies(3))
    ZERO[0] = 0
    wait(wb_copies(0))
    transpose_w(0, WT0, w_tiles)

    def first_group_dma(j):
        stages = (0, 2, 4, 7, 11, NT_J)
        if j in stages:
            wait(xp_copies(j, stages[stages.index(j) + 1]))
        if j == NT_J - 2:
            wait(wb_copies(1))

    def group(g, parity, first=False, last=False, dma=None):
        wt, wt_next = (WT0, WT1)[parity], (WT0, WT1)[1 - parity]
        act, act_prev = (ACT0, ACT1)[parity], (ACT0, ACT1)[1 - parity]
        tokens = (None, None)
        for j in range(NT_J):
            if dma is not None:
                dma(j)
            heads = []
            for t in range(3):
                tokens, prev = project(wt, act, j, t), tokens
                if first and j >= NT_J - 2:
                    transpose_w(1, wt_next, share(w_tiles, 6, 3 * (j - NT_J + 2) + t))
                if t == 0 and not first and not last:
                    transpose_w(g + 1, wt_next, share(w_tiles, NT_J, j))
                if not first:
                    heads += [attend_head(act_prev, j, hh, prev[when]) for hh, when in
                              (((0, 1),), ((1, 0),), ((2, 0), (3, 1)))[t]]
            if not first:
                store_heads(g - 1, j, heads)

    group(0, 0, first=True, dma=first_group_dma)

    def two_groups(i, carry):
        wait(wb_copies(2 * i + 2) + wb_copies(2 * i + 3))

        later = [c for g in range(4, NG) for c in wb_copies(g)] + wob_copies()
        for n, copies in enumerate((later + w_copies(0), w_copies(1) + awo_copies(),
                                    w_copies(2) + xa_copies() + [mem0_copy()])):
            pl.when(i == n)(functools.partial(start, copies))
        group(2 * i + 1, 1)
        group(2 * i + 2, 0)
        return carry

    lax.fori_loop(0, (NG - 2) // 2, two_groups, 0)
    group(NG - 1, 1, last=True)

    wait_all(WOB, sem_misc.at[0])
    wait_all(W, sem_misc.at[3])
    store_heads(NG - 1, 0, [attend_head(ACT1, 0, hh, None) for hh in range(4)])
    tokens = (None, None)
    w_items = list(range(3 * (NH // 2) * 8))
    for j in range(NT_J):
        heads = []
        for c in range(8):
            tokens, prev = project_out(j, c), tokens
            if j + 1 < NT_J and c % 2 == 0:
                heads.append(attend_head(ACT1, j + 1, c // 2, prev[0]))
            for item in share(w_items, NT_J * 8 - 4, j * 8 + c):
                split_heads(item, prev[item % 2])
        if heads:
            store_heads(NG - 1, j + 1, heads)
    start(outb_copies())

    wait_all(WO, sem_misc.at[1])
    wait_all(XA, sem_misc.at[2])
    mem0_copy().wait()
    for c in range(8):
        H[c, 0:MEM, :] = MEM0[:, c * 128:(c + 1) * 128].astype(f32)

    def segment(s):
        rows = pl.ds(pl.multiple_of(s * (SEG // 2), SEG // 2), SEG // 2)
        for c in range(8):
            H[c, MEM:ROWS, :] = _as_bf16(XA[c, rows, :]).astype(f32)
        h_in = jnp.concatenate([H[c] for c in range(8)], axis=1)

        def proj(t, h):
            return _mm(h_in, _as_bf16(W[3 * h + t]))

        def out_part(h0, h1, c):
            o = jnp.concatenate([OA[h] for h in range(h0, h1)], axis=1)
            return _mm(o, _as_bf16(WO[c, h0 * 64:h1 * 64, :]))

        def finish(pending):
            for h, (prob, v) in pending.items():
                OA[h] = _mm(prob, v)

        pending = {}
        for g in range(NH // HG):
            heads = range(g * HG, (g + 1) * HG)
            if g == 0:
                for h in heads:
                    HEAD[h] = _mm(h_in[:, :D // 2], _as_bf16(W[3 * h, 0:256, :]))
                q = {h: HEAD[h] + _mm(h_in[:, D // 2:], _as_bf16(W[3 * h, 256:512, :]))
                     for h in heads}
            else:
                q = {h: proj(0, h) for h in heads}
            k = {h: _a_keys(proj(1, h)) for h in heads}
            finish(pending)
            v = {h: _a_keys(proj(2, h)) for h in heads}
            pending = {h: (_a_probs(q[h], k[h]), v[h]) for h in heads}
        for c in range(4):
            PART[c] = out_part(0, NH // 2, c)
        finish(pending)
        for c in range(4, 8):
            PART[c] = out_part(0, NH // 2, c)
        for c in range(8):
            y = PART[c] + out_part(NH // 2, NH, c)
            H[c, 0:MEM, :] = y[0:MEM]
            OUTA[s, :, c * 128:(c + 1) * 128] = y[MEM:ROWS].astype(bf16)

    def step(p, carry):
        for u in range(UNROLL):
            segment(UNROLL * p + u)
        outa_copy(p).start()
        return carry

    lax.fori_loop(0, NSTEP, step, 0)

    wait_all(OUTB, sem_out.at[0])
    wait_all(OUTA, sem_out.at[1])


def _vmem(shape, dtype=i32):
    return pltpu.VMEM(shape, dtype)


@functools.partial(jax.jit, static_argnames=("A_seg_len",))
def pallas_concat_heads__memory_aug_recurrent_mem_tr__sliding_local_dilated__prompt_kernel(
    A_x: jax.Array,
    A_mem0: jax.Array,
    A_Wq: jax.Array,
    A_Wk: jax.Array,
    A_Wv: jax.Array,
    A_Wo: jax.Array,
    A_seg_len: int,
    B_x: jax.Array,
    B_wqkv: jax.Array,
    B_wo: jax.Array,
):
    assert A_seg_len == SEG and A_x.shape == (1, S, D) and A_mem0.shape == (1, MEM, D)
    assert A_Wq.shape == (D, NH, 128) and A_Wo.shape == (NH, 128, D)
    assert B_x.shape == (1, S, D) and B_wqkv.shape == (D, 3 * D) and B_wo.shape == (D, D)

    hbm = pl.BlockSpec(memory_space=pl.ANY)
    out = pl.pallas_call(
        _kernel,
        out_shape=jax.ShapeDtypeStruct((S // SEG, SEG, 2 * D), bf16),
        in_specs=[hbm] * 9,
        out_specs=hbm,
        scratch_shapes=[
            _vmem((3 * NH, 512, 128)),
            _vmem((8, 2048, 128)),
            _vmem((8, S // 2, 128)),
            _vmem((NT_J, 64, D)),
            _vmem((3 * NG, 512, 128)),
            _vmem((8, 192, 128)),
            _vmem((8, 192, 128)),
            _vmem((ACT_TILES, 128, 128), f32),
            _vmem((ACT_TILES, 128, 128), f32),
            _vmem((NT_J, NG, 64, 128)),
            _vmem((8, 512, 128)),
            _vmem((NT_J, 64, D)),
            _vmem((MEM, D), bf16),
            _vmem((8, ROWS, 128), f32),
            _vmem((NH, ROWS, 128), f32),
            _vmem((8, ROWS, 128), f32),
            _vmem((HG, ROWS, 128), f32),
            _vmem((S // SEG, SEG, D), bf16),
            pltpu.SMEM((1,), i32),
            pltpu.SemaphoreType.DMA((NT_J,)),
            pltpu.SemaphoreType.DMA((NG,)),
            pltpu.SemaphoreType.DMA((5,)),
            pltpu.SemaphoreType.DMA((2,)),
        ],
        compiler_params=pltpu.CompilerParams(vmem_limit_bytes=100 * 1024 * 1024),
    )(
        A_x.astype(bf16).reshape(S, D),
        A_mem0.astype(bf16).reshape(MEM, D),
        A_Wq.astype(bf16).reshape(D // 2, 2 * NH, 128),
        A_Wk.astype(bf16).reshape(D // 2, 2 * NH, 128),
        A_Wv.astype(bf16).reshape(D // 2, 2 * NH, 128),
        A_Wo.astype(bf16).reshape(NH * 128, D),
        B_x.astype(bf16).reshape(S // (2 * NT_J), 2 * NT_J, D),
        B_wqkv.astype(bf16),
        B_wo.astype(bf16),
    )
    return out.reshape(1, S, 2 * D)
```
